```python
import jax
import jax.numpy as jnp

def _softmax(x, axis=-1):
    return jax.nn.softmax(x, axis=axis)
def _gelu(x):
    return jax.nn.gelu(x, approximate=True)
def _silu(x):
    return jax.nn.silu(x)
def _sigmoid(x):
    return jax.nn.sigmoid(x)
def _layernorm(x, axis=-1, eps=1e-5):
    m = jnp.mean(x, axis=axis, keepdims=True)
    v = jnp.var(x, axis=axis, keepdims=True)
    return (x - m) / jnp.sqrt(v + eps)
def _scatter_add(tgt, idx, src, axis=0):
    return tgt.at[idx].add(src)
def _segment_sum(src, seg, n):
    return jax.ops.segment_sum(src, seg, n)
class _Rng:
    def __init__(self, key):
        self._k = key
    def _next(self):
        self._k, sub = jax.random.split(self._k)
        return sub
    def normal(self, shape):
        return jax.random.normal(self._next(), shape, dtype=jnp.bfloat16)
    def randint(self, lo, hi, shape):
        return jax.random.randint(self._next(), shape, lo, hi, dtype=jnp.int32)
    def uniform(self, shape, lo=0.0, hi=1.0):
        return jax.random.uniform(self._next(), shape, jnp.bfloat16, lo, hi)
    def permutation(self, n):
        return jax.random.permutation(self._next(), n)


kernel_name = 'concat_heads__sliding_local_dilated__ssm_conv_s4__prompt'

def setup_inputs():
    _rng = _Rng(jax.random.key(int.from_bytes(__import__("os").urandom(4), "little")))
    _w = (lambda a: (lambda t: t.astype(jnp.bfloat16) if jnp.issubdtype(t.dtype, jnp.floating) else t)(jnp.asarray(a)))
    def _A_setup():
        B, S, D = 1, 2048, 640
        return {
            "x": _w((lambda *s: _rng.normal(s) * 0.05)(B, S, D)),
            "wqkv": _w((lambda *s: _rng.normal(s) * 0.05)(D, 3 * D)),
            "wo": _w((lambda *s: _rng.normal(s) * 0.05)(D, D)),
        }
    _A_in = _A_setup()

    def _B_setup():
        B, L, D, N = 1, 2048, 640, 192
        A_re = -jnp.exp((lambda *s: _rng.normal(s) * 0.05)(D, N))
        A_im = jnp.pi * (lambda *s: _rng.normal(s) * 0.05)(D, N)
        B_re = (lambda *s: _rng.normal(s) * 0.05)(D, N)
        B_im = (lambda *s: _rng.normal(s) * 0.05)(D, N)
        C_re = (lambda *s: _rng.normal(s) * 0.05)(D, N)
        C_im = (lambda *s: _rng.normal(s) * 0.05)(D, N)
        log_dt = (lambda *s: _rng.normal(s) * 0.05)(D) * 0.5 - 4.0
        Dskip = (lambda *s: _rng.normal(s) * 0.05)(D)
        return {
            "u": _w((lambda *s: _rng.normal(s) * 0.05)(B, L, D)),
            "A_re": _w(A_re),
            "A_im": _w(A_im),
            "B_re": _w(B_re),
            "B_im": _w(B_im),
            "C_re": _w(C_re),
            "C_im": _w(C_im),
            "log_dt": _w(log_dt),
            "Dskip": _w(Dskip),
        }
    _B_in = _B_setup()

    return {
        "A_x": _A_in["x"],
        "A_wqkv": _A_in["wqkv"],
        "A_wo": _A_in["wo"],
        "B_u": _B_in["u"],
        "B_A_re": _B_in["A_re"],
        "B_A_im": _B_in["A_im"],
        "B_B_re": _B_in["B_re"],
        "B_B_im": _B_in["B_im"],
        "B_C_re": _B_in["C_re"],
        "B_C_im": _B_in["C_im"],
        "B_log_dt": _B_in["log_dt"],
        "B_Dskip": _B_in["Dskip"],
    }

def reference(A_x, A_wqkv, A_wo, B_u, B_A_re, B_A_im, B_B_re, B_B_im, B_C_re, B_C_im, B_log_dt, B_Dskip):
    def _A_ref(x, wqkv, wo):
        B, S, D = x.shape
        H = 32; Dh = D // H
        W, dil = 8, 2
        qkv = (lambda x, *d: x.transpose(*d))((x @ wqkv).reshape(B, S, 3, H, Dh), 2, 0, 3, 1, 4)
        q, k, v = qkv[0], qkv[1], qkv[2]
        scale = Dh ** -0.5
        pos = jnp.arange(S)
        off = jnp.arange(W) * dil
        idx = pos[:, None] - off[None, :]
        mask = idx >= 0
        idx_c = jnp.where(mask, idx, 0).reshape(-1)
        kg = k[:, :, idx_c, :].reshape(B, H, S, W, Dh)
        vg = v[:, :, idx_c, :].reshape(B, H, S, W, Dh)
        logits = jnp.einsum("bhsd,bhswd->bhsw", q, kg) * scale
        logits = jnp.where(mask[None, None, :, :], logits, -1e9)
        attn = _softmax(logits, axis=-1)
        o = jnp.einsum("bhsw,bhswd->bhsd", attn, vg)
        return (lambda x, *d: x.transpose(*d))(o, 0, 2, 1, 3).reshape(B, S, D) @ wo

    def _B_ref(u, A_re, A_im, B_re, B_im, C_re, C_im, log_dt, Dskip):
        Bsz, L, D = u.shape
        dt = jnp.exp(log_dt)[:, None]
        A = A_re + 1j * A_im
        Bc = B_re + 1j * B_im
        Cc = C_re + 1j * C_im
        logdA = dt * A
        dB = dt * Bc
        l = (lambda x, dt: x.astype(dt))(jnp.arange(L), A_re.dtype)
        P = jnp.exp(logdA[:, :, None] * l[None, None, :])
        K = jnp.einsum("dn,dnl,dn->dl", Cc, P, dB).real
        L2 = 2 * L
        Kp = jnp.pad(K, ((0, 0), (0, L)))
        up = (lambda x, *d: x.transpose(*d))(u, 0, 2, 1)
        up = jnp.pad(up, ((0, 0), (0, 0), (0, L)))
        Kf = (lambda x, axes=(-2,-1): jnp.fft.rfft2(x.astype(jnp.float32), axes=axes))(Kp[:, None, :], axes=(-2, -1))
        Uf = (lambda x, axes=(-2,-1): jnp.fft.rfft2(x.astype(jnp.float32), axes=axes))(up[:, :, None, :], axes=(-2, -1))
        Yf = Uf * Kf[None, :, :, :]
        y = (lambda x, s, axes=(-2,-1): jnp.fft.irfft2(x, s=s, axes=axes).astype(jnp.bfloat16))(Yf, (1, L2), axes=(-2, -1))[:, :, 0, :L]
        y = (lambda x, *d: x.transpose(*d))(y, 0, 2, 1) + u * Dskip[None, None, :]
        return y

    a = _A_ref(A_x, A_wqkv, A_wo)
    b = _B_ref(B_u, B_A_re, B_A_im, B_B_re, B_B_im, B_C_re, B_C_im, B_log_dt, B_Dskip)
    return jnp.concatenate([a, b], axis=-1)
```

```python
import functools

import jax
import jax.numpy as jnp
import ml_dtypes
import numpy as np
from jax import lax
import jax.experimental.pallas as pl
import jax.experimental.pallas.tpu as pltpu

S = 2048
D = 640
NT = D // 128
N = 192
H, DH = 32, 20
WIN, DIL = 8, 2
NB = S // 128
RB = 256
HALO = 16

F32 = jnp.float32
BF16 = jnp.bfloat16
NT_DIMS = (((1,), (1,)), ((), ()))

_ALPHA = ((1, 5, 2, 6), (3, 7, 4, 8), (258, 262, 260, 264), (516, 520, 772, 776),
          (1032, 1288, 1544, 1800))


@functools.lru_cache(maxsize=None)
def _tables():
    pos = {}
    for g in range(5):
        for b in range(32):
            for s in range(4):
                pos[_ALPHA[g][s] + 8 * b] = (g, (4 * b + s + 3) % 128)
    kk = np.concatenate([np.arange(0, 128, 2), np.arange(1, 128, 2)])
    th = 2 * np.pi * (kk + 0.5) / 256
    lr = np.arange(S, dtype=np.float32).astype(ml_dtypes.bfloat16).astype(np.int64)
    gm = {}
    for lag in range(1, S):
        m = (lag - 1) // 128
        g, j = pos[int(lr[lag])]
        gm.setdefault((m, g), np.zeros((128, 128), complex))[:, j] += np.exp(-1j * th * (lag - 128 * m))
    keys = tuple(sorted(gm))
    gt = np.stack([np.concatenate([gm[k].real, gm[k].imag]) for k in keys])
    f = np.exp(-1j * th[:, None] * np.arange(128)[None, :])
    fwd = np.concatenate([f.real, f.imag])
    inv = (2.0 / 256) * fwd.T
    cast = lambda a: np.asarray(a, np.float32).astype(ml_dtypes.bfloat16)
    return keys, cast(gt), cast(fwd), cast(inv)


def _cmul(a, b):
    return a[0] * b[0] - a[1] * b[1], a[0] * b[1] + a[1] * b[0]


def _ssm_operands(are, aim, bre, bim, cre, cim, dt, emit_p, emit_q):
    sub = lax.broadcasted_iota(jnp.int32, (8, 128), 0)
    low = sub < 4
    lr, li = dt * are, dt * aim
    w = _cmul((cre, cim), (dt * bre, dt * bim))
    ph = (jnp.cos(li), jnp.sin(li))
    pw = {}
    e = 1
    while e <= 1024:
        if e in (1, 4, 8, 16, 256, 512, 1024):
            mag = jnp.exp(lr * float(e))
            pw[e] = (mag * ph[0], mag * ph[1])
        if e < 1024:
            ph = (ph[0] * ph[0] - ph[1] * ph[1], 2.0 * ph[0] * ph[1])
        e *= 2
    w4 = _cmul(w, pw[4])
    w8 = _cmul(w, pw[8])
    w264 = _cmul(w8, pw[256])

    def swap(a):
        return tuple(pltpu.roll(v, 4, 0) for v in a)

    def sel(a, b):
        return tuple(jnp.where(low, x, y) for x, y in zip(a, b))

    def dup(a):
        s = swap(a)
        return sel(a, s), sel(s, a)

    def rev(a, cg):
        return tuple(jnp.take_along_axis(v, 4 * cg + 3 - sub % 4, axis=0) for v in a)

    z1, z256, z512, z1024 = (dup(pw[k]) for k in (1, 256, 512, 1024))
    z8, z16 = ((rev(pw[k], 0), rev(pw[k], 1)) for k in (8, 16))
    sw4, sw264 = swap(w4), swap(w264)
    p04 = (sel(w, sw4), sel(sw4, w))
    p8 = (sel(w8, sw264), sel(sw264, w8))
    one = (jnp.ones((8, 128), F32), jnp.zeros((8, 128), F32))
    q0 = (sel(one, z8[0]), sel(z8[1], z16[1]))
    for cg in range(2):
        p15 = _cmul(p04[cg], z1[cg])
        p26 = _cmul(p15, z1[cg])
        emit_p(cg, 0, p15, p26)
        p37 = _cmul(p26, z1[cg])
        p48 = _cmul(p37, z1[cg])
        emit_p(cg, 1, p37, p48)
        emit_p(cg, 2, _cmul(p26, z256[cg]), _cmul(p48, z256[cg]))
        p516 = _cmul(p48, z512[cg])
        emit_p(cg, 3, p516, _cmul(p516, z256[cg]))
        p1032 = _cmul(p8[cg], z1024[cg])
        emit_p(cg, 4, p1032, _cmul(p1032, z512[cg]))
        zc = (z16[cg][0], -z16[cg][1])
        q = [(q0[cg][0], -q0[cg][1])]
        for _ in range(15):
            q.append(_cmul(q[-1], zc))
        if cg == 1:
            q[15] = sel(q[15], one)
        for t in range(8):
            emit_q(cg, t, q[2 * t], q[2 * t + 1])


def _kernel(x_hbm, wqkv_hbm, wo_hbm, u_hbm, are_hbm, aim_hbm, bre_hbm, bim_hbm, cre_hbm, cim_hbm,
            ldt_ref, dsk_ref, g_hbm, f_hbm, fi_hbm, out_hbm,
            x_v, w_v, wo_v, u_v, par_v, g_v, f_v, fi_v, sems, osems,
            dt_v, gain_v, pa_v, qa_v, pb_v, qb_v, kt_v, uf_v, kf_v, yf_v,
            wt_v, wp_v, wot_v, wop_v, qkv_v, oa_v, ob_v, out_v):
    keys = _tables()[0]
    copies = [pltpu.make_async_copy(s_, par_v.at[i], sems.at[i]) for i, s_ in enumerate(
        (are_hbm, aim_hbm, bre_hbm, bim_hbm, cre_hbm, cim_hbm))]
    copies += [
        pltpu.make_async_copy(f_hbm, f_v, sems.at[6]),
        pltpu.make_async_copy(u_hbm.at[0], u_v, sems.at[7]),
        pltpu.make_async_copy(g_hbm, g_v, sems.at[8]),
        pltpu.make_async_copy(wqkv_hbm, w_v, sems.at[9]),
        pltpu.make_async_copy(wo_hbm, wo_v, sems.at[10]),
        pltpu.make_async_copy(x_hbm.at[0], x_v, sems.at[11]),
        pltpu.make_async_copy(fi_hbm, fi_v, sems.at[12]),
    ]
    for c in copies:
        c.start()

    dt_row = jnp.exp(ldt_ref[...].astype(F32)).astype(BF16).astype(F32)
    for t in range(NT):
        dt_v[128 * t:128 * (t + 1), :] = jnp.broadcast_to(dt_row[:, 128 * t:128 * (t + 1)], (128, 128)).T
    qkv_v[:, 0:HALO, :] = jnp.zeros((3 * NT, HALO, 128), F32)
    for c in copies[:6]:
        c.wait()

    for t in range(NT):
        rows = slice(128 * t, 128 * (t + 1))
        dt = dt_v[rows, :]
        b_re, b_im, c_re, c_im = (par_v[i, rows, :].astype(F32) for i in range(2, 6))
        wr = c_re * b_re - c_im * b_im
        k0 = jnp.sum(wr[:, :128], axis=1, keepdims=True) + jnp.sum(wr[:, 128:], axis=1, keepdims=True)
        k0 = (k0 * dt).T[0:8, :]
        gain_v[:, rows] = k0 + dsk_ref[:, rows].astype(F32)

    half = lax.broadcasted_iota(jnp.int32, (8, 128), 1) < 64

    def gen(i, p_ref, q_ref):
        rows = pl.ds(pl.multiple_of(i * 16, 16), 16)
        par = [par_v[k, rows, :].astype(F32) for k in range(6)]
        dt = dt_v[rows, :]

        def pack(a, b):
            return jnp.concatenate([a, b], axis=0).astype(BF16)

        for hf in range(2):
            def emit(ref, cg, t, a, b, hf=hf):
                ref[2 * hf + cg, 16 * t:16 * t + 16, 0:128] = pack(a[0], b[0])
                ref[2 * hf + cg, 16 * t:16 * t + 16, 128:256] = pack(a[1], b[1])
            r = slice(8 * hf, 8 * hf + 8)
            _ssm_operands(*[v[r, :128] for v in par], dt[r],
                          functools.partial(emit, p_ref), functools.partial(emit, q_ref))

        def emit2(ref, cg, t, a, b):
            re = pltpu.bitcast(pack(a[0], b[0]), jnp.uint32)
            im = pltpu.roll(pltpu.bitcast(pack(a[1], b[1]), jnp.uint32), 64, 1)
            ref[cg, 16 * t:16 * t + 16, 256:384] = pltpu.bitcast(jnp.where(half, re, im), BF16)
            ref[2 + cg, 16 * t:16 * t + 16, 256:384] = pltpu.bitcast(jnp.where(half, im, re), BF16)
        mix = [jnp.concatenate([v[0:8, 128:], v[8:16, 128:]], axis=1) for v in par]
        _ssm_operands(*mix, jnp.where(half, dt[0:8], dt[8:16]),
                      functools.partial(emit2, p_ref), functools.partial(emit2, q_ref))

    low = lax.broadcasted_iota(jnp.int32, (8, 128), 0) < 4
    slot = (lax.broadcasted_iota(jnp.int32, (8, 128), 1) + 1) % 4

    def kgen(i, p_ref, q_ref):
        for hf in range(2):
            o0, o1 = (lax.dot_general(p_ref[2 * hf + cg], q_ref[2 * hf + cg], NT_DIMS,
                                      preferred_element_type=F32) for cg in range(2))
            for g in range(5):
                parts = []
                for v in (2 * g, 2 * g + 1):
                    a, b = o0[8 * v:8 * v + 8], o1[8 * v:8 * v + 8]
                    parts += [jnp.where(low, a, b), pltpu.roll(jnp.where(low, b, a), 4, 0)]
                r = [pltpu.roll(p, s_, 1, stride=1, stride_axis=0) for s_, p in enumerate(parts)]
                r = jnp.where(slot < 2, jnp.where(slot == 0, r[0], r[1]), jnp.where(slot == 2, r[2], r[3]))
                kt_v[g, pl.ds(pl.multiple_of(i * 16 + 8 * hf, 8), 8), :] = r

    def udft(n):
        j, t = n // NT, n % NT
        blk = u_v[pl.ds(pl.multiple_of(j * 128, 128), 128), pl.ds(pl.multiple_of(t * 128, 128), 128)]
        uf_v[t, j] = jnp.dot(f_v[...], blk, preferred_element_type=F32)

    gen(0, pa_v, qa_v)
    copies[6].wait()
    copies[7].wait()

    def phase1(it, carry):
        gen(2 * it + 1, pb_v, qb_v)
        kgen(2 * it, pa_v, qa_v)
        udft(4 * it)
        udft(4 * it + 1)
        gen(jnp.minimum(2 * it + 2, D // 16 - 1), pa_v, qa_v)
        kgen(2 * it + 1, pb_v, qb_v)
        udft(4 * it + 2)
        udft(4 * it + 3)
        return carry
    lax.fori_loop(0, D // 32, phase1, 0)

    copies[8].wait()
    copies[9].wait()
    copies[10].wait()

    def phase2(t, carry):
        rows = pl.ds(pl.multiple_of(t * 128, 128), 128)
        kt = [kt_v[g, rows, :].astype(BF16) for g in range(5)]
        for m in range(NB):
            acc = None
            for idx, (mm, g) in enumerate(keys):
                if mm == m:
                    r = lax.dot_general(g_v[idx], kt[g], NT_DIMS, preferred_element_type=F32)
                    acc = r if acc is None else acc + r
            kf_v[t, m] = acc
        for c in range(3 * NT):
            wt_v[t, 128 * c:128 * (c + 1), :] = w_v[rows, 128 * c:128 * (c + 1)].astype(F32).T
        wot_v[t] = wo_v[:, rows].astype(F32)
        return carry
    lax.fori_loop(0, NT, phase2, 0)

    def permute(t, carry):
        cols = pl.ds(pl.multiple_of(t * 128, 128), 128)
        for part in range(3):
            for d in range(DH):
                r0 = part * D + d * H
                wp_v[r0:r0 + H, cols] = wt_v[t, pl.ds(part * D + d, H, stride=DH), :].astype(BF16)
        for d in range(DH):
            wop_v[d * H:(d + 1) * H, cols] = wot_v[t, pl.ds(d, H, stride=DH), :].astype(BF16)
        return carry
    lax.fori_loop(0, NT, permute, 0)

    copies[11].wait()
    scale = DH ** -0.5

    def block_products(t, r8, sg):
        re, im = pl.ds(r8, 8), pl.ds(r8 + 128, 8)
        prev = None
        for c in range(NB):
            yr = yi = None
            for j in range(c + 1):
                pr, pi = _cmul((kf_v[t, c - j, re, :], kf_v[t, c - j, im, :]),
                               (uf_v[t, j, re, :], uf_v[t, j, im, :]))
                yr, yi = (pr, pi) if yr is None else (yr + pr, yi + pi)
            if prev is None:
                yf_v[t, c, re, :] = yr
                yf_v[t, c, im, :] = yi
            else:
                yf_v[t, c, re, :] = yr - sg * prev[1]
                yf_v[t, c, im, :] = yi + sg * prev[0]
            prev = (yr, yi)

    def phase3(i, carry):
        r0 = pl.multiple_of(i * RB, RB)
        xb = x_v[pl.ds(r0, RB), :]
        for part in range(3):
            r = lax.dot_general(xb, wp_v[part * D:(part + 1) * D, :], NT_DIMS, preferred_element_type=F32)
            if part == 0:
                r = r * scale
            for t in range(NT):
                qkv_v[part * NT + t, pl.ds(r0 + HALO, RB), :] = r[:, 128 * t:128 * (t + 1)]
        sg = jnp.where(i < 4, 1.0, -1.0).astype(F32)
        for t in range(NT):
            for hf in range(2):
                block_products(t, pl.multiple_of(i * 16 + 8 * hf, 8), sg)
        return carry
    lax.fori_loop(0, S // RB, phase3, 0)

    copies[12].wait()

    def attend(i, o_ref):
        row = lax.broadcasted_iota(jnp.int32, (8, 128), 0)
        for sb in range(RB // 16):
            halves = []
            for hf in range(2):
                r = pl.multiple_of(i * RB + sb * 16 + hf * 8, 8)
                q = [qkv_v[t, pl.ds(r + HALO, 8), :] for t in range(NT)]
                lg = []
                for w in range(WIN):
                    src = pl.ds(r + (HALO - DIL * w), 8)
                    a = q[0] * qkv_v[NT, src, :]
                    for t in range(1, NT):
                        a = a + q[t] * qkv_v[NT + t, src, :]
                    a = a + pltpu.roll(a, 64, 1)
                    a = a + pltpu.roll(a, 32, 1)
                    if sb == 0 and w > 0:
                        a = jnp.where(row + r >= DIL * w, a, -1e9)
                    lg.append(a)
                mx = functools.reduce(jnp.maximum, lg)
                p = [jnp.exp(a - mx) for a in lg]
                inv = 1.0 / functools.reduce(lambda a, b: a + b, p)
                o = []
                for t in range(NT):
                    a = p[0] * qkv_v[2 * NT + t, pl.ds(r + HALO, 8), :]
                    for w in range(1, WIN):
                        a = a + p[w] * qkv_v[2 * NT + t, pl.ds(r + (HALO - DIL * w), 8), :]
                    o.append(a * inv)
                halves.append(o)
            for t in range(NT):
                o_ref[sb * 16:sb * 16 + 16, 128 * t:128 * (t + 1)] = jnp.concatenate(
                    [halves[0][t], halves[1][t]], axis=0).astype(BF16)

    def out_copy(i):
        rows = pl.ds(pl.multiple_of(i * RB, RB), RB)
        return pltpu.make_async_copy(out_v.at[rows, :], out_hbm.at[0, rows, :], osems.at[i])

    def finish(i, o_ref):
        r0 = pl.multiple_of(i * RB, RB)
        out_v[pl.ds(r0, RB), 0:D] = jnp.dot(o_ref[...], wop_v[...], preferred_element_type=F32).astype(BF16)
        for c2 in range(RB // 128):
            rows = pl.ds(pl.multiple_of(r0 + 128 * c2, 128), 128)
            for t in range(NT):
                cols = slice(128 * t, 128 * (t + 1))
                y = jnp.dot(fi_v[...], yf_v[t, i * (RB // 128) + c2].astype(BF16), preferred_element_type=F32)
                y = y + u_v[rows, cols].astype(F32) * gain_v[0:1, cols]
                out_v[rows, D + 128 * t:D + 128 * (t + 1)] = y.astype(BF16)
        out_copy(i).start()

    attend(0, oa_v)

    def phase4(it, carry):
        attend(2 * it + 1, ob_v)
        finish(2 * it, oa_v)
        attend(jnp.minimum(2 * it + 2, S // RB - 1), oa_v)
        finish(2 * it + 1, ob_v)
        return carry
    lax.fori_loop(0, S // RB // 2, phase4, 0)
    for i in range(S // RB):
        out_copy(i).wait()


@jax.jit
def pallas_concat_heads__sliding_local_dilated__ssm_conv_s4__prompt_kernel(
    A_x: jax.Array,
    A_wqkv: jax.Array,
    A_wo: jax.Array,
    B_u: jax.Array,
    B_A_re: jax.Array,
    B_A_im: jax.Array,
    B_B_re: jax.Array,
    B_B_im: jax.Array,
    B_C_re: jax.Array,
    B_C_im: jax.Array,
    B_log_dt: jax.Array,
    B_Dskip: jax.Array,
):
    keys, gt, fwd, inv = _tables()
    hbm = pl.BlockSpec(memory_space=pl.ANY)
    vmem = pl.BlockSpec(memory_space=pltpu.VMEM)
    scratch = [
        pltpu.VMEM((S, D), BF16),
        pltpu.VMEM((D, 3 * D), BF16),
        pltpu.VMEM((D, D), BF16),
        pltpu.VMEM((S, D), BF16),
        pltpu.VMEM((6, D, N), BF16),
        pltpu.VMEM(gt.shape, BF16),
        pltpu.VMEM(fwd.shape, BF16),
        pltpu.VMEM(inv.shape, BF16),
        pltpu.SemaphoreType.DMA((13,)),
        pltpu.SemaphoreType.DMA((S // RB,)),
        pltpu.VMEM((D, 128), F32),
        pltpu.VMEM((8, D), F32),
        pltpu.VMEM((4, 80, 384), BF16),
        pltpu.VMEM((4, 128, 384), BF16),
        pltpu.VMEM((4, 80, 384), BF16),
        pltpu.VMEM((4, 128, 384), BF16),
        pltpu.VMEM((5, D, 128), F32),
        pltpu.VMEM((NT, NB, 256, 128), F32),
        pltpu.VMEM((NT, NB, 256, 128), F32),
        pltpu.VMEM((NT, NB, 256, 128), F32),
        pltpu.VMEM((NT, 3 * D, 128), F32),
        pltpu.VMEM((3 * D, D), BF16),
        pltpu.VMEM((NT, D, 128), F32),
        pltpu.VMEM((D, D), BF16),
        pltpu.VMEM((3 * NT, S + HALO, 128), F32),
        pltpu.VMEM((RB, D), BF16),
        pltpu.VMEM((RB, D), BF16),
        pltpu.VMEM((S, 2 * D), BF16),
    ]
    return pl.pallas_call(
        _kernel,
        in_specs=[hbm] * 10 + [vmem, vmem] + [hbm] * 3,
        out_specs=hbm,
        out_shape=jax.ShapeDtypeStruct((1, S, 2 * D), BF16),
        scratch_shapes=scratch,
        compiler_params=pltpu.CompilerParams(vmem_limit_bytes=110 * 2**20),
    )(A_x, A_wqkv, A_wo, B_u, B_A_re, B_A_im, B_B_re, B_B_im, B_C_re, B_C_im,
      B_log_dt.reshape(1, D), B_Dskip.reshape(1, D), gt, fwd, inv)
```

```python
import functools

import jax
import jax.numpy as jnp
import ml_dtypes
import numpy as np
from jax import lax
import jax.experimental.pallas as pl
import jax.experimental.pallas.tpu as pltpu

S = 2048
D = 640
NT = D // 128
N = 192
H, DH = 32, 20
WIN, DIL = 8, 2
NB = S // 128
RB = 256
HALO = 16

F32 = jnp.float32
BF16 = jnp.bfloat16
U32 = jnp.uint32
NT_DIMS = (((1,), (1,)), ((), ()))

_ALPHA = ((1, 5, 2, 6), (3, 7, 4, 8), (258, 262, 260, 264), (516, 520, 772, 776),
          (1032, 1288, 1544, 1800))


@functools.lru_cache(maxsize=None)
def _tables():
    pos = {}
    for g in range(5):
        for b in range(32):
            for s in range(4):
                pos[_ALPHA[g][s] + 8 * b] = (g, (4 * b + s + 3) % 128)
    kk = np.concatenate([np.arange(0, 128, 2), np.arange(1, 128, 2)])
    th = 2 * np.pi * (kk + 0.5) / 256
    lr = np.arange(S, dtype=np.float32).astype(ml_dtypes.bfloat16).astype(np.int64)
    gm = {}
    for lag in range(1, S):
        m = (lag - 1) // 128
        g, j = pos[int(lr[lag])]
        gm.setdefault((m, g), np.zeros((128, 128), complex))[:, j] += np.exp(-1j * th * (lag - 128 * m))
    keys = tuple(sorted(gm))
    gt = np.stack([np.concatenate([gm[k].real, gm[k].imag]) for k in keys])
    f = np.exp(-1j * th[:, None] * np.arange(128)[None, :])
    fwd = np.concatenate([f.real, f.imag])
    inv = (2.0 / 256) * fwd.T

    def words(a):
        b = np.asarray(a, np.float32).astype(ml_dtypes.bfloat16).view(np.uint16).astype(np.uint32)
        return b[..., 0::2, :] | (b[..., 1::2, :] << 16)
    return keys, words(gt), words(fwd), words(np.stack([inv[:, :128], inv[:, 128:]]))


def _cmul(a, b):
    return a[0] * b[0] - a[1] * b[1], a[0] * b[1] + a[1] * b[0]


def _interleave(main, n_main, side, n_side):
    done = 0
    for k, _ in enumerate(main):
        while done * n_main < (k + 1) * n_side:
            next(side, None)
            done += 1
        yield
    _run(side)


def _run(gen):
    for _ in gen:
        pass


def _chain(*gens):
    for g in gens:
        yield from g


def _pack(a, b):
    return jnp.concatenate([a, b], axis=0).astype(BF16)


def _rows(ref, idx, start, size):
    start = start // 2 if isinstance(start, int) else pl.multiple_of(start // 2, 8)
    return pltpu.bitcast(ref.bitcast(U32)[(*idx, pl.ds(start, size // 2), slice(None))], BF16)


UF0, KT0, BASE0 = 0, NT * NB * 256, NT * NB * 256 + 5 * D
Z_ROWS = BASE0 + 3 * 28 * 8
KF0 = NT * S
GATE0 = KF0 + NT * NB * 256
BIG_ROWS = GATE0 + 8 * (S // RB)


def _kernel(x_hbm, wqkv_hbm, wo_hbm, u_hbm, are_hbm, aim_hbm, bre_hbm, bim_hbm, cre_hbm, cim_hbm,
            ldt_ref, dsk_ref, g_hbm, f_hbm, fi_hbm, out_hbm,
            x_v, w_v, wo_v, u_v, par_v, g_v, f_v, fi_v, sems, osems,
            lo_v, hi_v, gain_v, pa_v, pa3_v, qa_v, qa3_v, pb_v, pb3_v, qb_v, qb3_v, tmp_v, z_v, big_v, yf_v,
            wt_v, wp_v, wot_v, wop_v, oa_v, ob_v, out_v, lg0_v, lg1_v, kv_v):
    keys = _tables()[0]
    bufa, bufb = ((pa_v, pa3_v), (qa_v, qa3_v)), ((pb_v, pb3_v), (qb_v, qb3_v))
    par_cp = [pltpu.make_async_copy(s_, par_v.at[i], sems.at[i]) for i, s_ in enumerate(
        (are_hbm, aim_hbm, bre_hbm, bim_hbm, cre_hbm, cim_hbm))]
    f_cp = pltpu.make_async_copy(f_hbm, f_v, sems.at[6])

    def u_cp(i):
        cols = pl.ds(pl.multiple_of(i * 128, 128), 128)
        return pltpu.make_async_copy(u_hbm.at[0, :, cols], u_v.at[i], sems.at[7 + i])
    late_cp = [pltpu.make_async_copy(a_, b_, sems.at[12 + i]) for i, (a_, b_) in enumerate(
        ((g_hbm, g_v), (wqkv_hbm, w_v), (wo_hbm, wo_v), (fi_hbm, fi_v))
        + tuple((x_hbm.at[0, :, 128 * t:128 * (t + 1)], x_v.at[t]) for t in range(NT)))]
    for c in par_cp + [f_cp] + [u_cp(i) for i in range(NT)] + late_cp:
        c.start()

    kv_v[:, 0:HALO, :] = jnp.zeros((2 * NT, HALO, 128), F32)
    dt = jnp.exp(ldt_ref[...].astype(F32)).astype(BF16).astype(F32).reshape(1, D)
    for c in par_cp:
        c.wait()
    a_re, a_im, b_re, b_im, c_re, c_im = (par_v[i].astype(F32) for i in range(6))
    w_re, w_im = _cmul((c_re, c_im), (dt * b_re, dt * b_im))
    gain_v[...] = jnp.sum(w_re, axis=0, keepdims=True) + dsk_ref[...].astype(F32).reshape(1, D)
    for k, v in enumerate((dt * a_re, dt * a_im, w_re, w_im)):
        for t in range(NT):
            lo_v[k, 128 * t:128 * (t + 1), :] = v[0:128, 128 * t:128 * (t + 1)].T
        y = jnp.concatenate([v[128:, 0:384], jnp.concatenate([v[128:, D // 2:], v[128:, 0:64]], axis=1)], axis=0)
        for t in range(3):
            hi_v[k, 128 * t:128 * (t + 1), :] = y[:, 128 * t:128 * (t + 1)].T

    sub = lax.broadcasted_iota(jnp.int32, (8, 128), 0)
    lane = lax.broadcasted_iota(jnp.int32, (8, 128), 1)
    low, half, slot = sub < 4, lane < 64, (lane + 1) % 4

    def sel(a, b):
        return tuple(jnp.where(low, x, y) for x, y in zip(a, b))

    def bases(slab, lr, li, w):
        ph = (jnp.cos(li), jnp.sin(li))
        pw = {}
        e = 1
        while e <= 1024:
            if e in (1, 4, 8, 16, 256, 512, 1024):
                mag = jnp.exp(lr * float(e))
                pw[e] = (mag * ph[0], mag * ph[1])
            if e < 1024:
                ph = (ph[0] * ph[0] - ph[1] * ph[1], 2.0 * ph[0] * ph[1])
            e *= 2
        w8 = _cmul(w, pw[8])

        def pair(a, b):
            sb = tuple(pltpu.roll(v, 4, 0) for v in b)
            return sel(a, sb), sel(sb, a)

        def rev(a, cg):
            re, im = (jnp.take_along_axis(v, 4 * cg + 3 - sub % 4, axis=0) for v in a)
            return re, -im

        one = (jnp.ones((8, 128), F32), jnp.zeros((8, 128), F32))
        z16 = (rev(pw[16], 0), rev(pw[16], 1))
        vals = [pair(pw[k], pw[k]) for k in (1, 256, 512, 1024)]
        vals += [pair(w, _cmul(w, pw[4])), pair(w8, _cmul(w8, pw[256])), z16,
                 (sel(one, rev(pw[8], 0)), sel(rev(pw[8], 1), z16[1]))]
        for k, v in enumerate(vals[:7]):
            for cg in range(2):
                for c in range(2):
                    r = BASE0 + 8 * (28 * slab + 4 * k + 2 * cg + c)
                    z_v[r:r + 8, :] = v[cg][c]
        return vals[7]

    def powers(slab, q0, emit_p, emit_q):
        for cg in range(2):
            def ld(k):
                r = BASE0 + 8 * (28 * slab + 4 * k + 2 * cg)
                return z_v[r:r + 8, :], z_v[r + 8:r + 16, :]
            z = ld(0)
            p15 = _cmul(ld(4), z)
            p26 = _cmul(p15, z)
            emit_p(cg, 0, p15, p26)
            yield
            z = ld(0)
            p37 = _cmul(p26, z)
            p48 = _cmul(p37, z)
            emit_p(cg, 1, p37, p48)
            yield
            z = ld(1)
            emit_p(cg, 2, _cmul(p26, z), _cmul(p48, z))
            yield
            p516 = _cmul(p48, ld(2))
            emit_p(cg, 3, p516, _cmul(p516, ld(1)))
            yield
            p1032 = _cmul(ld(5), ld(3))
            emit_p(cg, 4, p1032, _cmul(p1032, ld(2)))
            yield
            qb = None
            for t in range(8):
                z = ld(6)
                qa = q0[cg] if t == 0 else _cmul(qb, z)
                qb = _cmul(qa, z)
                if cg == 1 and t == 7:
                    qb = sel(qb, (1.0, 0.0))
                emit_q(cg, t, qa, qb)
                yield

    def gen(i, p_ref, q_ref):
        q0 = []
        for slab in range(3):
            src = hi_v if slab == 2 else lo_v
            rows = pl.ds(pl.multiple_of(i * 8 + (D // 2 if slab == 1 else 0), 8), 8)
            q0.append(bases(slab, src[0, rows, :], src[1, rows, :], (src[2, rows, :], src[3, rows, :])))
            yield
        for hf in range(2):
            def emit(ref, cg, t, a, b, hf=hf):
                ref[2 * hf + cg, 0, 16 * t:16 * t + 16, :] = _pack(a[0], b[0])
                ref[2 * hf + cg, 1, 16 * t:16 * t + 16, :] = _pack(a[1], b[1])
            yield from powers(hf, q0[hf], functools.partial(emit, p_ref[0]), functools.partial(emit, q_ref[0]))

        n = [0]

        def emit2(ref, cg, t, a, b):
            tmp_v[n[0], 0] = _pack(a[0], b[0])
            tmp_v[n[0], 1] = _pack(a[1], b[1])
            re = tmp_v.bitcast(U32)[n[0], 0]
            im = pltpu.roll(tmp_v.bitcast(U32)[n[0], 1], 64, 1)
            n[0] += 1
            ref[1][cg, 8 * t:8 * t + 8, :] = jnp.where(half, re, im)
            ref[1][2 + cg, 8 * t:8 * t + 8, :] = jnp.where(half, im, re)
        yield from powers(2, q0[2], functools.partial(emit2, p_ref), functools.partial(emit2, q_ref))
    n_gen = 3 + 3 * 26

    def words(ref, *idx):
        return jnp.concatenate([pltpu.bitcast(ref[(*idx, k)], BF16) for k in range(ref.shape[len(idx)])], axis=1)

    def kgen(i, hf, p_ref, q_ref):
        def operand(ref, grp, size):
            return jnp.concatenate([_rows(ref[0], (grp, 0), 0, size), _rows(ref[0], (grp, 1), 0, size),
                                    pltpu.bitcast(ref[1][grp], BF16)], axis=1)
        o0, o1 = (lax.dot_general(operand(p_ref, 2 * hf + cg, 80), operand(q_ref, 2 * hf + cg, 128), NT_DIMS,
                                  preferred_element_type=F32) for cg in range(2))
        for g in range(5):
            parts = []
            for v in (2 * g, 2 * g + 1):
                a, b = o0[8 * v:8 * v + 8], o1[8 * v:8 * v + 8]
                parts += [jnp.where(low, a, b), pltpu.roll(jnp.where(low, b, a), 4, 0)]
            r = [pltpu.roll(p, s_, 1, stride=1, stride_axis=0) for s_, p in enumerate(parts)]
            r = jnp.where(slot < 2, jnp.where(slot == 0, r[0], r[1]), jnp.where(slot == 2, r[2], r[3]))
            z_v[pl.ds(pl.multiple_of(KT0 + g * D + hf * (D // 2) + i * 8, 8), 8), :] = r
            yield

    def udft(n):
        t, j = n // NB, n % NB
        r = jnp.dot(pltpu.bitcast(f_v[...], BF16), _rows(u_v, (t,), j * 128, 128), preferred_element_type=F32)
        for q in range(0, 256, 16):
            z_v[pl.ds(pl.multiple_of(UF0 + (t * NB + j) * 256 + q, 16), 16), :] = r[q:q + 16]
            yield

    _run(gen(0, *bufa))
    f_cp.wait()
    n_it = D // 32

    def phase1(it, carry):
        @pl.when(it % (n_it // NT) == 0)
        def _():
            u_cp(it // (n_it // NT)).wait()
        for i, cur, nxt in ((2 * it, bufa, bufb), (2 * it + 1, bufb, bufa)):
            mxu = _chain(kgen(i, 0, *cur), udft(2 * i), kgen(i, 1, *cur), udft(2 * i + 1))
            _run(_interleave(mxu, 42, gen(jnp.minimum(i + 1, 2 * n_it - 1), *nxt), n_gen))
        return carry
    with jax.named_scope("phase1"):
        lax.fori_loop(0, n_it, phase1, 0)

    for c in late_cp:
        c.wait()

    def phase2(t, carry):
        rows = pl.ds(pl.multiple_of(t * 128, 128), 128)
        kt = [z_v[pl.ds(pl.multiple_of(KT0 + g * D + t * 128, 128), 128), :].astype(BF16) for g in range(5)]
        for m in range(NB):
            acc = None
            for idx, (mm, g) in enumerate(keys):
                if mm == m:
                    r = lax.dot_general(pltpu.bitcast(g_v[idx], BF16), kt[g], NT_DIMS, preferred_element_type=F32)
                    acc = r if acc is None else acc + r
            big_v[pl.ds(pl.multiple_of(KF0 + (t * NB + m) * 256, 8), 256), :] = acc
        for c in range(3 * NT):
            wt_v[128 * c:128 * (c + 1), :] = w_v[rows, 128 * c:128 * (c + 1)].astype(F32).T
        wot_v[...] = wo_v[:, rows].astype(F32)
        for d in range(DH):
            for part in range(3):
                r0 = part * D + d * H
                wp_v[t, r0:r0 + H, :] = wt_v[pl.ds(part * D + d, H, stride=DH), :].astype(BF16)
            wop_v[t, d * H:(d + 1) * H, :] = wot_v[pl.ds(d, H, stride=DH), :].astype(BF16)
        return carry
    with jax.named_scope("phase2"):
        lax.fori_loop(0, NT, phase2, 0)

    scale = DH ** -0.5

    def block_products(t, r8, sg):
        def ld(ref, base, m):
            r = pl.multiple_of(base + (t * NB + m) * 256 + r8, 8)
            return ref[pl.ds(r, 8), :], ref[pl.ds(r + 128, 8), :]
        prev = None
        for c0 in range(0, NB, 2):
            acc, kc = [None, None], {}
            for j in range(c0 + 1, -1, -1):
                u = ld(z_v, UF0, j)
                for c in range(c0 + 1, max(c0, j) - 1, -1):
                    if c - j not in kc:
                        kc[c - j] = ld(big_v, KF0, c - j)
                    p, a = _cmul(kc[c - j], u), acc[c - c0]
                    acc[c - c0] = p if a is None else (a[0] + p[0], a[1] + p[1])
                    yield
            for c in (c0, c0 + 1):
                yr, yi = acc[c - c0]
                if prev is not None:
                    yr, yi = yr - sg * prev[1], yi + sg * prev[0]
                yf_v[t, c, pl.ds(r8, 8), :] = yr
                yf_v[t, c, pl.ds(r8 + 128, 8), :] = yi
                prev = acc[c - c0]

    def qkv(r0):
        for n in range(3 * NT):
            xb = jnp.concatenate([_rows(x_v, (k,), r0, RB) for k in range(NT)], axis=1)
            w = jnp.concatenate([_rows(wp_v, (k,), 128 * n, 128) for k in range(NT)], axis=1)
            r = lax.dot_general(xb, w, NT_DIMS, preferred_element_type=F32)
            for q in range(0, RB, 16):
                if n < NT:
                    big_v[pl.ds(pl.multiple_of(n * S + r0 + q, 8), 16), :] = r[q:q + 16] * scale
                else:
                    kv_v[n - NT, pl.ds(pl.multiple_of(HALO + r0 + q, 8), 16), :] = r[q:q + 16]
                    big_v[pl.ds(pl.multiple_of(GATE0 + r0 // 32, 8), 8), :] = r[q:q + 8]
                yield

    def logits(i):
        lag = 3
        for step in range(RB // 8 + lag):
            n = step
            if n < RB // 8:
                r = pl.multiple_of(i * RB + n * 8, 8)
                q = [big_v[pl.ds(t * S + r, 8), :] for t in range(NT)]
                for w in range(WIN):
                    src = pl.ds(r + HALO - DIL * w, 8)
                    a = q[0] * kv_v[0, src, :]
                    for t in range(1, NT):
                        a = a + q[t] * kv_v[t, src, :]
                    lg0_v[(n * WIN + w) * 8:(n * WIN + w + 1) * 8, :] = a
            n = step - lag
            if n >= 0:
                for w in range(WIN):
                    a = lg0_v[(n * WIN + w) * 8:(n * WIN + w + 1) * 8, :]
                    lg1_v[pl.ds(pl.multiple_of(i * RB * WIN + (n * WIN + w) * 8, 8), 8), :] = (
                        a + pltpu.roll(a, 64, 1))
            yield

    def phase3(i, carry):
        sg = jnp.where(i < 4, 1.0, -1.0).astype(F32)
        prod = _chain(*[block_products(t, pl.multiple_of(i * 16 + 8 * hf, 8), sg)
                        for t in range(NT) for hf in range(2)])
        side = _interleave(prod, 10 * 136, logits(jnp.maximum(i - 1, 0)), RB // 8 + 3)
        _run(_interleave(qkv(pl.multiple_of(i * RB, RB)), 3 * NT * RB // 16, side, 10 * 136))
        return carry
    with jax.named_scope("phase3"):
        lax.fori_loop(0, S // RB, phase3, 0)

    def attend(i, o_ref):
        def softmax(n):
            r = pl.multiple_of(i * RB + n * 8, 8)
            sc = []
            for w in range(WIN):
                a = lg1_v[pl.ds(pl.multiple_of(i * RB * WIN + (n * WIN + w) * 8, 8), 8), :]
                a = a + pltpu.roll(a, 32, 1)
                if n * 8 < DIL * w:
                    a = jnp.where(sub + r >= DIL * w, a, -1e9)
                sc.append(a)
            mx = functools.reduce(jnp.maximum, sc)
            p = [jnp.exp(a - mx) for a in sc]
            inv = 1.0 / functools.reduce(lambda a, b: a + b, p)
            for w in range(WIN):
                lg0_v[(n * WIN + w) * 8:(n * WIN + w + 1) * 8, :] = p[w] * inv

        held, lag = None, 3
        for n in range(-lag, RB // 8):
            if n + lag < RB // 8:
                softmax(n + lag)
            yield
            if n < 0:
                continue
            r = pl.multiple_of(i * RB + n * 8, 8)
            p = [lg0_v[(n * WIN + w) * 8:(n * WIN + w + 1) * 8, :] for w in range(WIN)]
            o = []
            for t in range(NT):
                a = p[0] * kv_v[NT + t, pl.ds(r + HALO, 8), :]
                for w in range(1, WIN):
                    a = a + p[w] * kv_v[NT + t, pl.ds(r + HALO - DIL * w, 8), :]
                o.append(a)
            if n % 2 == 0:
                held = o
            else:
                for t in range(NT):
                    o_ref[t, 8 * (n - 1):8 * (n + 1), :] = _pack(held[t], o[t])
            yield
    n_att = 2 * RB // 8 + 3

    def out_copy(i):
        rows = pl.ds(pl.multiple_of(i * RB, RB), RB)
        return pltpu.make_async_copy(out_v.at[rows, :], out_hbm.at[0, rows, :], osems.at[i])

    def finish(i, o_ref):
        r0 = pl.multiple_of(i * RB, RB)

        def gate(v):
            for ref, base in ((lg0_v, WIN * RB), (lg1_v, WIN * S)):
                ref[pl.ds(pl.multiple_of(base + 8 * i, 8), 8), :] = v
        for t in range(NT):
            r = jnp.dot(jnp.concatenate([_rows(o_ref, (k,), 0, RB) for k in range(NT)], axis=1),
                        _rows(wop_v, (t,), 0, D), preferred_element_type=F32)
            for q in range(0, RB, 16):
                out_v[pl.ds(r0 + q, 16), 128 * t:128 * (t + 1)] = r[q:q + 16].astype(BF16)
                gate(r[q:q + 8])
                yield
            cols = slice(128 * t, 128 * (t + 1))
            for c2 in range(RB // 128):
                y = jnp.dot(words(fi_v), yf_v[t, i * (RB // 128) + c2].astype(BF16), preferred_element_type=F32)
                for q in range(0, 128, 32):
                    rows = pl.ds(pl.multiple_of(r0 + 128 * c2 + q, 32), 32)
                    yq = y[q:q + 32] + u_v[t, rows, :].astype(F32) * gain_v[:, cols]
                    out_v[rows, D + 128 * t:D + 128 * (t + 1)] = yq.astype(BF16)
                    gate(yq[0:8])
                    yield
    n_fin = NT * (RB // 16 + 4 * RB // 128)

    _run(logits(S // RB - 1))
    _run(attend(0, oa_v))

    def phase4(it, carry):
        _run(_interleave(finish(2 * it, oa_v), n_fin, attend(2 * it + 1, ob_v), n_att))
        out_copy(2 * it).start()
        _run(_interleave(finish(2 * it + 1, ob_v), n_fin, attend(jnp.minimum(2 * it + 2, S // RB - 1), oa_v), n_att))
        out_copy(2 * it + 1).start()
        return carry
    with jax.named_scope("phase4"):
        lax.fori_loop(0, S // RB // 2, phase4, 0)
    for i in range(S // RB):
        out_copy(i).wait()


@jax.jit
def pallas_concat_heads__sliding_local_dilated__ssm_conv_s4__prompt_kernel(
    A_x: jax.Array,
    A_wqkv: jax.Array,
    A_wo: jax.Array,
    B_u: jax.Array,
    B_A_re: jax.Array,
    B_A_im: jax.Array,
    B_B_re: jax.Array,
    B_B_im: jax.Array,
    B_C_re: jax.Array,
    B_C_im: jax.Array,
    B_log_dt: jax.Array,
    B_Dskip: jax.Array,
):
    keys, gt, fwd, inv = _tables()
    hbm = pl.BlockSpec(memory_space=pl.ANY)
    vmem = pl.BlockSpec(memory_space=pltpu.VMEM)
    scratch = [
        pltpu.VMEM((NT, S, 128), BF16),
        pltpu.VMEM((D, 3 * D), BF16),
        pltpu.VMEM((D, D), BF16),
        pltpu.VMEM((NT, S, 128), BF16),
        pltpu.VMEM((6, N, D), BF16),
        pltpu.VMEM(gt.shape, U32),
        pltpu.VMEM(fwd.shape, U32),
        pltpu.VMEM(inv.shape, U32),
        pltpu.SemaphoreType.DMA((21,)),
        pltpu.SemaphoreType.DMA((S // RB,)),
        pltpu.VMEM((4, D, 128), F32),
        pltpu.VMEM((4, 384, 128), F32),
        pltpu.VMEM((1, D), F32),
        pltpu.VMEM((4, 2, 80, 128), BF16),
        pltpu.VMEM((4, 40, 128), U32),
        pltpu.VMEM((4, 2, 128, 128), BF16),
        pltpu.VMEM((4, 64, 128), U32),
        pltpu.VMEM((4, 2, 80, 128), BF16),
        pltpu.VMEM((4, 40, 128), U32),
        pltpu.VMEM((4, 2, 128, 128), BF16),
        pltpu.VMEM((4, 64, 128), U32),
        pltpu.VMEM((26, 2, 16, 128), BF16),
        pltpu.VMEM((Z_ROWS, 128), F32),
        pltpu.VMEM((BIG_ROWS, 128), F32),
        pltpu.VMEM((NT, NB, 256, 128), F32),
        pltpu.VMEM((3 * D, 128), F32),
        pltpu.VMEM((NT, 3 * D, 128), BF16),
        pltpu.VMEM((D, 128), F32),
        pltpu.VMEM((NT, D, 128), BF16),
        pltpu.VMEM((NT, RB, 128), BF16),
        pltpu.VMEM((NT, RB, 128), BF16),
        pltpu.VMEM((S, 2 * D), BF16),
        pltpu.VMEM((WIN * RB + 64, 128), F32),
        pltpu.VMEM((WIN * S + 64, 128), F32),
        pltpu.VMEM((2 * NT, S + HALO, 128), F32),
    ]
    return pl.pallas_call(
        _kernel,
        in_specs=[hbm] * 10 + [vmem, vmem] + [hbm] * 3,
        out_specs=hbm,
        out_shape=jax.ShapeDtypeStruct((1, S, 2 * D), BF16),
        scratch_shapes=scratch,
        compiler_params=pltpu.CompilerParams(vmem_limit_bytes=110 * 2**20),
    )(A_x, A_wqkv, A_wo, B_u, B_A_re.T, B_A_im.T, B_B_re.T, B_B_im.T, B_C_re.T, B_C_im.T,
      B_log_dt, B_Dskip, gt, fwd, inv)
```

```python
import functools

import jax
import jax.numpy as jnp
import ml_dtypes
import numpy as np
from jax import lax
import jax.experimental.pallas as pl
import jax.experimental.pallas.tpu as pltpu

S = 2048
D = 640
NT = D // 128
N = 192
H, DH = 32, 20
WIN, DIL = 8, 2
NB = S // 128
RB = 256
NBK = 1
LOG2E = float(np.log2(np.e))
HALO = 16

F32 = jnp.float32
BF16 = jnp.bfloat16
U32 = jnp.uint32
NT_DIMS = (((1,), (1,)), ((), ()))

_ALPHA = ((1, 5, 2, 6), (3, 7, 4, 8), (258, 262, 260, 264), (516, 520, 772, 776),
          (1032, 1288, 1544, 1800))


@functools.lru_cache(maxsize=None)
def _tables():
    pos = {}
    for g in range(5):
        for b in range(32):
            for s in range(4):
                pos[_ALPHA[g][s] + 8 * b] = (g, (4 * b + s + 3) % 128)
    kk = np.concatenate([np.arange(0, 128, 2), np.arange(1, 128, 2)])
    th = 2 * np.pi * (kk + 0.5) / 256
    lr = np.arange(S, dtype=np.float32).astype(ml_dtypes.bfloat16).astype(np.int64)
    gm = {}
    for lag in range(1, S):
        m = (lag - 1) // 128
        g, j = pos[int(lr[lag])]
        gm.setdefault((m, g), np.zeros((128, 128), complex))[:, j] += np.exp(-1j * th * (lag - 128 * m))
    keys = tuple(sorted(gm))

    gt = np.stack([np.concatenate([gm[k].real, gm[k].imag]) for k in keys])
    f = np.exp(-1j * th[:, None] * np.arange(128)[None, :])
    fwd = np.concatenate([f.real, f.imag])
    inv = (2.0 / 256) * np.concatenate([f.real, f.imag]).T

    def words(a):
        b = np.asarray(a, np.float32).astype(ml_dtypes.bfloat16).view(np.uint16).astype(np.uint32)
        return b[..., 0::2, :] | (b[..., 1::2, :] << 16)
    return keys, words(gt), words(fwd), words(np.stack([inv[:, :128], inv[:, 128:]]))


def _cmul(a, b):
    return a[0] * b[0] - a[1] * b[1], a[0] * b[1] + a[1] * b[0]


def _interleave(main, n_main, side, n_side, lead=0):
    for _ in range(lead):
        next(side)
    n_side -= lead
    done = 0
    for k, _ in enumerate(main):
        while done * n_main < (k + 1) * n_side:
            next(side, None)
            done += 1
        yield
    _run(side)


def _take(gen, n):
    for _ in range(n):
        next(gen, None)
        yield


def _run(gen):
    for _ in gen:
        pass


def _chain(*gens):
    for g in gens:
        yield from g


def _pack(a, b):
    return jnp.concatenate([a, b], axis=0).astype(BF16)


def _rows(ref, idx, start, size):
    start = start // 2 if isinstance(start, int) else pl.multiple_of(start // 2, 8)
    return pltpu.bitcast(ref.bitcast(U32)[(*idx, pl.ds(start, size // 2), slice(None))], BF16)


SLABS = 3 * D // 2
KF0 = NT * S
GATE0 = KF0 + NT * NB * 256
BIG_ROWS = GATE0 + 8 * (S // RB)


def _kernel(x_hbm, wqkv_hbm, wo_hbm, u_hbm, are_hbm, aim_hbm, bre_hbm, bim_hbm, cre_hbm, cim_hbm,
            ldt_ref, dsk_ref, g_hbm, f_hbm, fi_hbm, out_hbm,
            x_v, w_v, wo_v, u_v, par_v, g_v, f_v, fi_v, sems, osems, zero_s,
            gain_v, rawa_v, rawb_v, tmp_v, kt_v, base_v, z_v, uf_v, big_v, yf_v,
            wt_v, wp_v, wop_v, oa_v, ob_v, out_v, lg0_v, lg1_v, k_v, v_v, *pq_refs):
    keys = _tables()[0]
    zero_s[0] = 0
    par_cp = [pltpu.make_async_copy(s_, par_v.at[i], sems.at[i]) for i, s_ in enumerate(
        (are_hbm, aim_hbm, bre_hbm, bim_hbm, cre_hbm, cim_hbm))]
    f_cp = pltpu.make_async_copy(f_hbm, f_v, sems.at[6])

    def u_cp(i):
        cols = pl.ds(pl.multiple_of(i * 128, 128), 128)
        return pltpu.make_async_copy(u_hbm.at[0, :, cols], u_v.at[i], sems.at[7 + i])
    late_cp = [pltpu.make_async_copy(a_, b_, sems.at[12 + i]) for i, (a_, b_) in enumerate(
        ((g_hbm, g_v), (wqkv_hbm, w_v), (wo_hbm, wo_v), (fi_hbm, fi_v))
        + tuple((x_hbm.at[0, :, 128 * t:128 * (t + 1)], x_v.at[t]) for t in range(NT)))]
    for c in par_cp + [f_cp] + [u_cp(i) for i in range(NT)] + late_cp:
        c.start()

    k_v[:, 0:HALO, :] = v_v[:, 0:HALO, :] = jnp.zeros((NT, HALO, 128), F32)
    dt = jnp.exp(ldt_ref[...].astype(F32)).astype(BF16).astype(F32).reshape(1, D)
    for c in par_cp:
        c.wait()
    a_re, a_im, b_re, b_im, c_re, c_im = (par_v[i].astype(F32) for i in range(6))
    w_re, w_im = _cmul((c_re, c_im), (dt * b_re, dt * b_im))
    gain_v[...] = jnp.sum(w_re, axis=0, keepdims=True) + dsk_ref[...].astype(F32).reshape(1, D)
    for k, v in enumerate((dt * a_re, dt * a_im, w_re, w_im)):
        for t in range(NT):
            r = k * SLABS + 192 * t
            vt = v[:, 128 * t:128 * (t + 1)]
            z_v[r:r + 128, :] = vt[0:128].T
            hi = vt[128:].T
            z_v[r + 128:r + 192, :] = jnp.concatenate([hi[0:64], hi[64:128]], axis=1)

    sub = lax.broadcasted_iota(jnp.int32, (8, 128), 0)
    lane = lax.broadcasted_iota(jnp.int32, (8, 128), 1)
    low, half, slot = sub < 4, lane < 64, (lane + 1) % 4

    def sel(a, b):
        return tuple(jnp.where(low, x, y) for x, y in zip(a, b))

    def bases(r0, nv):
        def par(k):
            return z_v[pl.ds(pl.multiple_of(k * SLABS + r0, 8), 8 * nv), :]

        def put(k, fn, *args):
            for n in range(nv):
                v = fn(*[tuple(c[8 * n:8 * n + 8] for c in a) for a in args])
                for cg in range(2):
                    for c in range(2):
                        r = 32 * (r0 + 8 * n) + 8 * (4 * k + 2 * c + cg)
                        base_v[pl.ds(pl.multiple_of(r, 8), 8), :] = v[cg][c]

        def pair(a, b):
            sb = tuple(pltpu.roll(v, 4, 0) for v in b)
            return sel(a, sb), sel(sb, a)

        def rev(a):
            return [tuple(jnp.take_along_axis(v, 4 * cg + 3 - sub % 4, axis=0) for v in (a[0], -a[1]))
                    for cg in range(2)]

        def first(z8, z16):
            z8 = rev(z8)
            return sel((1.0, 0.0), z8[0]), sel(z8[1], rev(z16)[1])

        li = par(1)
        ph = (jnp.cos(li), jnp.sin(li))
        pw = {}
        e = 1
        while e <= 1024:
            if e in (1, 4, 8, 16, 256, 512, 1024):
                yield
                mag = jnp.exp(par(0) * float(e))
                pw[e] = (mag * ph[0], mag * ph[1])
            if e in (1, 256, 512, 1024):
                put((1, 256, 512, 1024).index(e), pair, pw[e], pw[e])
            if e == 4:
                w = (par(2), par(3))
                put(4, pair, w, _cmul(w, pw[4]))
            if e == 16:
                put(6, rev, pw[16])
                put(7, first, pw[8], pw[16])
            if e == 256:
                w8 = _cmul((par(2), par(3)), pw[8])
                put(5, pair, w8, _cmul(w8, pw[256]))
            if e < 1024:
                ph = (ph[0] * ph[0] - ph[1] * ph[1], 2.0 * ph[0] * ph[1])
            e *= 2

    def powers(i, slab, emit):
        def ld(k):
            r = pl.multiple_of(32 * (192 * (i // 8) + 64 * slab + 8 * (i % 8)) + 32 * k, 8)
            return base_v[pl.ds(r, 16), :], base_v[pl.ds(r + 16, 16), :]
        z = ld(0)
        p15 = _cmul(ld(4), z)
        yield
        p26 = _cmul(p15, ld(0))
        emit(0, p15, p26)
        yield
        p37 = _cmul(p26, ld(0))
        yield
        p48 = _cmul(p37, ld(0))
        emit(1, p37, p48)
        yield
        z = ld(1)
        emit(2, _cmul(p26, z), _cmul(p48, z))
        yield
        p516 = _cmul(p48, ld(2))
        yield
        emit(3, p516, _cmul(p516, ld(1)))
        yield
        p1032 = _cmul(ld(5), ld(3))
        yield
        emit(4, p1032, _cmul(p1032, ld(2)))
        yield
        qb = None
        for t in range(8):
            qa = ld(7) if t == 0 else _cmul(qb, ld(6))
            yield
            qb = _cmul(qa, ld(6))
            if t == 7:
                keep = lax.broadcasted_iota(jnp.int32, (16, 128), 0) < 12
                qb = (jnp.where(keep, qb[0], 1.0), jnp.where(keep, qb[1], 0.0))
            emit(5 + t, qa, qb)
            yield

    def gen(i, pq_v, pq3_v):
        for hf in range(2):
            def emit(t, a, b, hf=hf):
                for cg in range(2):
                    for c in range(2):
                        pq_v[2 * hf + cg, c, 16 * t:16 * t + 16, :] = _pack(
                            a[c][8 * cg:8 * cg + 8], b[c][8 * cg:8 * cg + 8])
            yield from powers(i, hf, emit)

        def emit2(t, a, b):
            for cg in range(2):
                n = 13 * cg + t
                for c in range(2):
                    tmp_v[n, c] = _pack(a[c][8 * cg:8 * cg + 8], b[c][8 * cg:8 * cg + 8])
                re = tmp_v.bitcast(U32)[n, 0]
                im = pltpu.roll(tmp_v.bitcast(U32)[n, 1], 64, 1)
                pq3_v[cg, 8 * t:8 * t + 8, :] = jnp.where(half, re, im)
                pq3_v[2 + cg, 8 * t:8 * t + 8, :] = jnp.where(half, im, re)
        yield from powers(i, 2, emit2)

    def kgen(hf, pq_v, pq3_v, raw_v, zero, gate):
        def operand(grp, start, size):
            return jnp.concatenate(
                [_rows(pq_v, (grp, 0), start, size), _rows(pq_v, (grp, 1), start, size),
                 pltpu.bitcast(pq3_v[grp, start // 2:(start + size) // 2, :], BF16)], axis=1)
        outs = [lax.dot_general(operand(zero + 2 * hf + cg, 0, 80), operand(zero + 2 * hf + cg, 80, 128), NT_DIMS,
                                preferred_element_type=F32) for cg in range(2)]
        for cg, o in enumerate(outs):
            for g in range(5):
                r = 80 * (2 * hf + cg) + 16 * g
                raw_v[r:r + 16, :] = o[16 * g:16 * g + 16]
                gate(o[16 * g:16 * g + 8])
                yield

    def extract(i, raw_v):
        for hf in range(2):
            for g in range(5):
                parts = []
                for v in (2 * g, 2 * g + 1):
                    a, b = (raw_v[80 * (2 * hf + cg) + 8 * v:80 * (2 * hf + cg) + 8 * v + 8, :] for cg in range(2))
                    parts += [jnp.where(low, a, b), pltpu.roll(jnp.where(low, b, a), 4, 0)]
                r = [pltpu.roll(p, s_, 1, stride=1, stride_axis=0) for s_, p in enumerate(parts)]
                r = jnp.where(slot < 2, jnp.where(slot == 0, r[0], r[1]), jnp.where(slot == 2, r[2], r[3]))
                kt_v[g, pl.ds(pl.multiple_of(128 * (i // 8) + 64 * hf + 8 * (i % 8), 8), 8), :] = r

    def udft(t, j):
        r = jnp.dot(pltpu.bitcast(f_v[...], BF16), _rows(u_v, (t,), j * 128, 128), preferred_element_type=F32)
        for q in range(0, 256, 64):
            uf_v[pl.ds(pl.multiple_of((t * NB + j) * 256 + q, 8), 64), :] = r[q:q + 64]
            z_v[pl.ds(pl.multiple_of(zero_s[0] + 4 * SLABS, 8), 8), :] = r[q:q + 8]
            yield

    def kdft(t, gate):
        rows = pl.ds(pl.multiple_of(t * 128, 128), 128)
        for m in range(NB):
            acc = None
            for idx, (mm, g) in enumerate(keys):
                if mm == m:
                    r = lax.dot_general(pltpu.bitcast(g_v[idx], BF16), kt_v[g, rows, :].astype(BF16), NT_DIMS,
                                        preferred_element_type=F32)
                    acc = r if acc is None else acc + r
            for q in range(0, 256, 64):
                big_v[pl.ds(pl.multiple_of(KF0 + (t * NB + m) * 256 + q, 8), 64), :] = acc[q:q + 64]
                gate(acc[q:q + 8])
                yield

    def weights(t, k):
        rows = pl.ds(pl.multiple_of(t * 128, 128), 128)
        if k < 3:
            for c in range(NT):
                wt_v[k, 128 * c:128 * (c + 1), :] = w_v[rows, k * D + 128 * c:k * D + 128 * (c + 1)].astype(F32).T
        elif k == 3:
            wt_v[3] = wo_v[:, rows].astype(F32)
        else:
            for d in range(DH):
                v = wt_v[k - 4, pl.ds(d, H, stride=DH), :].astype(BF16)
                if k < 7:
                    wp_v[t, (k - 4) * D + d * H:(k - 4) * D + (d + 1) * H, :] = v
                else:
                    wop_v[t, d * H:(d + 1) * H, :] = v

    f_cp.wait()

    def phase0(t, carry):
        u_cp(t).wait()
        mxu = _chain(*[udft(t, j) for j in range(NB)])
        side = _chain(*[bases(192 * t + 24 * c, 3) for c in range(8)])
        _run(_interleave(mxu, 4 * NB, side, 8 * 7, lead=2))
        return carry
    with jax.named_scope("phase0"):
        lax.fori_loop(0, NT, phase0, 0)

    n_grp = D // 16
    bufs = list(zip(pq_refs[0::2], pq_refs[1::2]))
    raws = (rawa_v, rawb_v)
    _run(gen(0, *bufs[0]))
    _run(gen(1, *bufs[1]))
    for c in late_cp:
        c.wait()

    def phase1(t, carry):
        zero = zero_s[0]

        def gate(v):
            base_v[pl.ds(pl.multiple_of(zero + 32 * SLABS, 8), 8), :] = v
        dft = kdft(jnp.maximum(t - 1, 0), gate)
        for k in range(8):
            i = 8 * t + k
            extract(jnp.maximum(i - 1, 0), raws[(k + 1) % 2])
            weights(t, k)
            n_dft = (0, 8, 8, 8, 8, 8, 12, 12)[k]
            mxu = _chain(kgen(0, *bufs[k % 4], raws[k % 2], zero, gate), _take(dft, n_dft // 2),
                         kgen(1, *bufs[k % 4], raws[k % 2], zero, gate), _take(dft, n_dft // 2))
            side = gen(jnp.minimum(i + 2, n_grp - 1), *bufs[(k + 2) % 4])
            _run(_interleave(mxu, 20 + n_dft, side, 75, lead=20 if k == 0 else 0))
        return carry
    with jax.named_scope("phase1"):
        lax.fori_loop(0, NT, phase1, 0)
    extract(n_grp - 1, raws[(n_grp - 1) % 2])
    _run(kdft(NT - 1, lambda v: None))

    scale = DH ** -0.5 * LOG2E

    def block_products(t, r8, sg):
        def ld(ref, base, m):
            return [ref[pl.ds(pl.multiple_of(base + ((t * NB + m) * 2 + c) * 128 + r8, 8), 8), :] for c in range(2)]
        prev = None
        for c0 in range(0, NB, 2):
            acc, kc = [None, None], {}
            for j in range(c0 + 1, -1, -1):
                u = ld(uf_v, 0, j)
                for c in range(c0 + 1, max(c0, j) - 1, -1):
                    if c - j not in kc:
                        kc[c - j] = ld(big_v, KF0, c - j)
                    p, a = _cmul(kc[c - j], u), acc[c - c0]
                    acc[c - c0] = p if a is None else [x + y for x, y in zip(a, p)]
                    yield
            for c in (c0, c0 + 1):
                cur = yr, yi = acc[c - c0]
                if prev is not None:
                    yr, yi = yr - sg * prev[1], yi + sg * prev[0]
                yf_v[t, c, pl.ds(r8, 8), :] = yr
                yf_v[t, c, pl.ds(r8 + 128, 8), :] = yi
                prev = cur

    def qkv(r0):
        for n0 in range(0, 3 * NT, NBK):
            xb = jnp.concatenate([_rows(x_v, (k,), r0, RB) for k in range(NT)], axis=1)
            w = jnp.concatenate([_rows(wp_v, (k,), 128 * n0, 128 * NBK) for k in range(NT)], axis=1)
            r = lax.dot_general(xb, w, NT_DIMS, preferred_element_type=F32)
            for q in range(0, RB, 16):
                for n in range(n0, n0 + NBK):
                    v = r[q:q + 16, 128 * (n - n0):128 * (n - n0 + 1)]
                    if n < NT:
                        big_v[pl.ds(pl.multiple_of(n * S + r0 + q, 8), 16), :] = v * scale
                    elif n < 2 * NT:
                        k_v[n % NT, pl.ds(pl.multiple_of(HALO + r0 + q, 8), 16), :] = v
                    else:
                        v_v[n % NT, pl.ds(pl.multiple_of(HALO + r0 + q, 8), 16), :] = v
                        big_v[pl.ds(pl.multiple_of(GATE0 + r0 // 32, 8), 8), :] = v[0:8]
                    yield

    def logits(i):
        lag = 3
        for step in range(RB // 8 + lag):
            n = step
            if n < RB // 8:
                r = pl.multiple_of(i * RB + n * 8, 8)
                a = [None] * WIN
                for t in range(NT):
                    q = big_v[pl.ds(t * S + r, 8), :]
                    for w in range(WIN):
                        qk = q * k_v[t, pl.ds(r + HALO - DIL * w, 8), :]
                        a[w] = qk if t == 0 else a[w] + qk
                    yield
                for w in range(WIN):
                    lg0_v[(n * WIN + w) * 8:(n * WIN + w + 1) * 8, :] = a[w]
            n = step - lag
            if n >= 0:
                for w in range(WIN):
                    a = lg0_v[(n * WIN + w) * 8:(n * WIN + w + 1) * 8, :]
                    lg1_v[pl.ds(pl.multiple_of(i * RB * WIN + (n * WIN + w) * 8, 8), 8), :] = (
                        a + pltpu.roll(a, 64, 1))
            yield

    def phase3(i, carry):
        sg = jnp.where(i < 4, 1.0, -1.0).astype(F32)
        prod = _chain(*[block_products(t, pl.multiple_of(i * 16 + 8 * hf, 8), sg)
                        for t in range(NT) for hf in range(2)])
        lgt, mxu = logits(jnp.maximum(i - 1, 0)), qkv(pl.multiple_of(i * RB, RB))
        n_mxu, n_lgt = NT * RB // 16, 3 * RB // 8 + 2
        for n_prod in (380, 600, 380):
            side = _take(prod, n_prod)
            if n_prod < 600:
                side = _interleave(side, n_prod, _take(lgt, n_lgt), n_lgt)
            _run(_interleave(_take(mxu, n_mxu), n_mxu, side, n_prod))
        _run(_chain(mxu, prod, lgt))
        return carry
    with jax.named_scope("phase3"):
        lax.fori_loop(0, S // RB, phase3, 0)

    def attend(i, o_ref):
        def softmax(n):
            r = pl.multiple_of(i * RB + n * 8, 8)
            sc = []
            for w in range(WIN):
                a = lg1_v[pl.ds(pl.multiple_of(i * RB * WIN + (n * WIN + w) * 8, 8), 8), :]
                a = a + pltpu.roll(a, 32, 1)
                if n * 8 < DIL * w:
                    a = jnp.where(sub + r >= DIL * w, a, -1e9 * LOG2E)
                sc.append(a)
            mx = functools.reduce(jnp.maximum, sc)
            p = [jnp.exp2(a - mx) for a in sc]
            inv = 1.0 / functools.reduce(lambda a, b: a + b, p)
            o = [None] * NT
            for w in range(WIN):
                for t in range(NT):
                    pv = p[w] * v_v[t, pl.ds(r + HALO - DIL * w, 8), :]
                    o[t] = pv if w == 0 else o[t] + pv
            return [v * inv for v in o]

        held = None
        for n in range(RB // 8):
            o = softmax(n)
            if n % 2 == 0:
                held = o
            else:
                for t in range(NT):
                    o_ref[t, 8 * (n - 1):8 * (n + 1), :] = _pack(held[t], o[t])
            yield
    n_att = RB // 8

    def out_copy(i):
        rows = pl.ds(pl.multiple_of(i * RB, RB), RB)
        return pltpu.make_async_copy(out_v.at[rows, :], out_hbm.at[0, rows, :], osems.at[i])

    def finish(i, o_ref):
        r0 = pl.multiple_of(i * RB, RB)

        def gate(v):
            for ref, base in ((lg1_v, WIN * S),):
                ref[pl.ds(pl.multiple_of(base + 8 * i, 8), 8), :] = v
        for t in range(NT):
            r = jnp.dot(jnp.concatenate([_rows(o_ref, (k,), 0, RB) for k in range(NT)], axis=1),
                        _rows(wop_v, (t,), 0, D), preferred_element_type=F32)
            for q in range(0, RB, 16):
                out_v[pl.ds(r0 + q, 16), 128 * t:128 * (t + 1)] = r[q:q + 16].astype(BF16)
                gate(r[q:q + 8])
                yield
            cols = slice(128 * t, 128 * (t + 1))
            for c2 in range(RB // 128):
                fi = jnp.concatenate([pltpu.bitcast(fi_v[k], BF16) for k in range(2)], axis=1)
                y = jnp.dot(fi, yf_v[t, i * (RB // 128) + c2].astype(BF16), preferred_element_type=F32)
                for q in range(0, 128, 32):
                    rows = pl.ds(pl.multiple_of(r0 + 128 * c2 + q, 32), 32)
                    yq = y[q:q + 32] + u_v[t, rows, :].astype(F32) * gain_v[:, cols]
                    out_v[rows, D + 128 * t:D + 128 * (t + 1)] = yq.astype(BF16)
                    gate(yq[0:8])
                    yield
    n_fin = NT * (RB // 16 + 4 * RB // 128)

    _run(logits(S // RB - 1))
    _run(attend(0, oa_v))

    def phase4(it, carry):
        _run(_interleave(finish(2 * it, oa_v), n_fin, attend(2 * it + 1, ob_v), n_att))
        out_copy(2 * it).start()
        _run(_interleave(finish(2 * it + 1, ob_v), n_fin, attend(jnp.minimum(2 * it + 2, S // RB - 1), oa_v), n_att))
        out_copy(2 * it + 1).start()
        return carry
    with jax.named_scope("phase4"):
        lax.fori_loop(0, S // RB // 2, phase4, 0)
    for i in range(S // RB):
        out_copy(i).wait()


@jax.jit
def pallas_concat_heads__sliding_local_dilated__ssm_conv_s4__prompt_kernel(
    A_x: jax.Array,
    A_wqkv: jax.Array,
    A_wo: jax.Array,
    B_u: jax.Array,
    B_A_re: jax.Array,
    B_A_im: jax.Array,
    B_B_re: jax.Array,
    B_B_im: jax.Array,
    B_C_re: jax.Array,
    B_C_im: jax.Array,
    B_log_dt: jax.Array,
    B_Dskip: jax.Array,
):
    keys, gt, fwd, inv = _tables()
    hbm = pl.BlockSpec(memory_space=pl.ANY)
    vmem = pl.BlockSpec(memory_space=pltpu.VMEM)
    scratch = [
        pltpu.VMEM((NT, S, 128), BF16),
        pltpu.VMEM((D, 3 * D), BF16),
        pltpu.VMEM((D, D), BF16),
        pltpu.VMEM((NT, S, 128), BF16),
        pltpu.VMEM((6, N, D), BF16),
        pltpu.VMEM(gt.shape, U32),
        pltpu.VMEM(fwd.shape, U32),
        pltpu.VMEM(inv.shape, U32),
        pltpu.SemaphoreType.DMA((21,)),
        pltpu.SemaphoreType.DMA((S // RB,)),
        pltpu.SMEM((1,), jnp.int32),
        pltpu.VMEM((1, D), F32),
        pltpu.VMEM((320, 128), F32),
        pltpu.VMEM((320, 128), F32),
        pltpu.VMEM((26, 2, 16, 128), BF16),
        pltpu.VMEM((5, D, 128), F32),
        pltpu.VMEM((32 * SLABS + 8, 128), F32),
        pltpu.VMEM((4 * SLABS + 8, 128), F32),
        pltpu.VMEM((NT * NB * 256, 128), F32),
        pltpu.VMEM((BIG_ROWS, 128), F32),
        pltpu.VMEM((NT, NB, 256, 128), F32),
        pltpu.VMEM((4, D, 128), F32),
        pltpu.VMEM((NT, 3 * D, 128), BF16),
        pltpu.VMEM((NT, D, 128), BF16),
        pltpu.VMEM((NT, RB, 128), BF16),
        pltpu.VMEM((NT, RB, 128), BF16),
        pltpu.VMEM((S, 2 * D), BF16),
        pltpu.VMEM((WIN * RB + 64, 128), F32),
        pltpu.VMEM((WIN * S + 64, 128), F32),
        pltpu.VMEM((NT, S + HALO, 128), F32),
        pltpu.VMEM((NT, S + HALO, 128), F32),
    ] + 4 * [
        pltpu.VMEM((4, 2, 208, 128), BF16),
        pltpu.VMEM((4, 104, 128), U32),
    ]
    return pl.pallas_call(
        _kernel,
        in_specs=[hbm] * 10 + [vmem, vmem] + [hbm] * 3,
        out_specs=hbm,
        out_shape=jax.ShapeDtypeStruct((1, S, 2 * D), BF16),
        scratch_shapes=scratch,
        compiler_params=pltpu.CompilerParams(vmem_limit_bytes=110 * 2**20),
    )(A_x, A_wqkv, A_wo, B_u, B_A_re.T, B_A_im.T, B_B_re.T, B_B_im.T, B_C_re.T, B_C_im.T,
      B_log_dt, B_Dskip, gt, fwd, inv)
```

```python
import functools

import jax
import jax.numpy as jnp
import ml_dtypes
import numpy as np
from jax import lax
import jax.experimental.pallas as pl
import jax.experimental.pallas.tpu as pltpu

S = 2048
D = 640
NT = D // 128
N = 192
H, DH = 32, 20
WIN, DIL = 8, 2
NB = S // 128
RB = 256
NBK = 1
LOG2E = float(np.log2(np.e))
HALO = 16

F32 = jnp.float32
BF16 = jnp.bfloat16
U32 = jnp.uint32
NT_DIMS = (((1,), (1,)), ((), ()))

_ALPHA = ((1, 5, 2, 6), (3, 7, 4, 8), (258, 262, 260, 264), (516, 520, 772, 776),
          (1032, 1288, 1544, 1800))


@functools.lru_cache(maxsize=None)
def _tables():
    pos = {}
    for g in range(5):
        for b in range(32):
            for s in range(4):
                pos[_ALPHA[g][s] + 8 * b] = (g, (4 * b + s + 3) % 128)
    kk = np.concatenate([np.arange(0, 128, 2), np.arange(1, 128, 2)])
    th = 2 * np.pi * (kk + 0.5) / 256
    lr = np.arange(S, dtype=np.float32).astype(ml_dtypes.bfloat16).astype(np.int64)
    gm = {}
    for lag in range(1, S):
        m = (lag - 1) // 128
        g, j = pos[int(lr[lag])]
        gm.setdefault((m, g), np.zeros((128, 128), complex))[:, j] += np.exp(-1j * th * (lag - 128 * m))
    keys = tuple(sorted(gm))

    gt = np.stack([np.concatenate([gm[k].real, gm[k].imag]) for k in keys])
    f = np.exp(-1j * th[:, None] * np.arange(128)[None, :])
    fwd = np.concatenate([f.real, f.imag])
    inv = (2.0 / 256) * np.concatenate([f.real, f.imag]).T

    def words(a):
        b = np.asarray(a, np.float32).astype(ml_dtypes.bfloat16).view(np.uint16).astype(np.uint32)
        return b[..., 0::2, :] | (b[..., 1::2, :] << 16)
    return keys, words(gt), words(fwd), words(np.stack([inv[:, :128], inv[:, 128:]]))


def _cmul(a, b):
    return a[0] * b[0] - a[1] * b[1], a[0] * b[1] + a[1] * b[0]


def _interleave(main, n_main, side, n_side, lead=0):
    for _ in range(lead):
        next(side)
    n_side -= lead
    done = 0
    for k, _ in enumerate(main):
        while done * n_main < (k + 1) * n_side:
            next(side, None)
            done += 1
        yield
    _run(side)


def _take(gen, n):
    for _ in range(n):
        next(gen, None)
        yield


def _run(gen):
    for _ in gen:
        pass


def _chain(*gens):
    for g in gens:
        yield from g


def _pack(a, b):
    return jnp.concatenate([a, b], axis=0).astype(BF16)


def _rows(ref, idx, start, size):
    start = start // 2 if isinstance(start, int) else pl.multiple_of(start // 2, 8)
    return pltpu.bitcast(ref.bitcast(U32)[(*idx, pl.ds(start, size // 2), slice(None))], BF16)


SLABS = 3 * D // 2
KF0 = NT * S
GATE0 = KF0 + NT * NB * 256
BIG_ROWS = GATE0 + 8 * (S // RB)


def _kernel(x_hbm, wqkv_hbm, wo_hbm, u_hbm, are_hbm, aim_hbm, bre_hbm, bim_hbm, cre_hbm, cim_hbm,
            ldt_ref, dsk_ref, g_hbm, f_hbm, fi_hbm, out_hbm,
            x_v, w_v, wo_v, u_v, par_v, g_v, f_v, fi_v, sems, osems, zero_s,
            gain_v, rawa_v, rawb_v, tmp_v, kt_v, base_v, z_v, uf_v, big_v, yf_v,
            wt_v, wp_v, wop_v, oa_v, ob_v, out_v, lg0_v, lg1_v, k_v, v_v, *pq_refs):
    keys = _tables()[0]
    zero_s[0] = 0

    def par_cp(t):
        cols = pl.ds(pl.multiple_of(t * 128, 128), 128)
        return [pltpu.make_async_copy(s_.at[:, cols], par_v.at[t, i], sems.at[t]) for i, s_ in enumerate(
            (are_hbm, aim_hbm, bre_hbm, bim_hbm, cre_hbm, cim_hbm))]
    f_cp = pltpu.make_async_copy(f_hbm, f_v, sems.at[6])

    def u_cp(i):
        cols = pl.ds(pl.multiple_of(i * 128, 128), 128)
        return pltpu.make_async_copy(u_hbm.at[0, :, cols], u_v.at[i], sems.at[7 + i])
    late_cp = [pltpu.make_async_copy(a_, b_, sems.at[12 + i]) for i, (a_, b_) in enumerate(
        ((g_hbm, g_v), (wqkv_hbm, w_v), (wo_hbm, wo_v), (fi_hbm, fi_v))
        + tuple((x_hbm.at[0, :, 128 * t:128 * (t + 1)], x_v.at[t]) for t in range(NT)))]
    for c in par_cp(0) + [f_cp, u_cp(0)] + par_cp(1):
        c.start()

    k_v[:, 0:HALO, :] = v_v[:, 0:HALO, :] = jnp.zeros((NT, HALO, 128), F32)
    dt_row = jnp.exp(ldt_ref[...].astype(F32)).astype(BF16).astype(F32).reshape(1, D)
    skip_row = dsk_ref[...].astype(F32).reshape(1, D)
    for t in range(NT):
        gain_v[t, 0:1, :] = dt_row[:, 128 * t:128 * (t + 1)]
        gain_v[t, 1:2, :] = skip_row[:, 128 * t:128 * (t + 1)]

    def prepare(t):
        dt = gain_v[t, 0:1, :]
        a_re, a_im, b_re, b_im, c_re, c_im = (par_v[t, i].astype(F32) for i in range(6))
        w_re, w_im = _cmul((c_re, c_im), (dt * b_re, dt * b_im))
        gain_v[t, 2:3, :] = jnp.sum(w_re, axis=0, keepdims=True) + gain_v[t, 1:2, :]
        for k, v in enumerate((dt * a_re, dt * a_im, w_re, w_im)):
            r = pl.multiple_of(k * SLABS + 192 * t, 8)
            z_v[pl.ds(r, 128), :] = v[0:128].T
            hi = v[128:].T
            z_v[pl.ds(r + 128, 64), :] = jnp.concatenate([hi[0:64], hi[64:128]], axis=1)

    for c in par_cp(0):
        c.wait()
    for t in range(1, NT):
        for c in [u_cp(t)] + (par_cp(t + 1) if t + 1 < NT else []):
            c.start()
    prepare(0)

    sub = lax.broadcasted_iota(jnp.int32, (8, 128), 0)
    lane = lax.broadcasted_iota(jnp.int32, (8, 128), 1)
    low, half, slot = sub < 4, lane < 64, (lane + 1) % 4

    def sel(a, b):
        return tuple(jnp.where(low, x, y) for x, y in zip(a, b))

    def bases(r0, nv):
        def par(k):
            return z_v[pl.ds(pl.multiple_of(k * SLABS + r0, 8), 8 * nv), :]

        def put(k, fn, *args):
            for n in range(nv):
                v = fn(*[tuple(c[8 * n:8 * n + 8] for c in a) for a in args])
                for cg in range(2):
                    for c in range(2):
                        r = 32 * (r0 + 8 * n) + 8 * (4 * k + 2 * c + cg)
                        base_v[pl.ds(pl.multiple_of(r, 8), 8), :] = v[cg][c]

        def pair(a, b):
            sb = tuple(pltpu.roll(v, 4, 0) for v in b)
            return sel(a, sb), sel(sb, a)

        def rev(a):
            return [tuple(jnp.take_along_axis(v, 4 * cg + 3 - sub % 4, axis=0) for v in (a[0], -a[1]))
                    for cg in range(2)]

        def first(z8, z16):
            z8 = rev(z8)
            return sel((1.0, 0.0), z8[0]), sel(z8[1], rev(z16)[1])

        li = par(1)
        ph = (jnp.cos(li), jnp.sin(li))
        pw = {}
        e = 1
        while e <= 1024:
            if e in (1, 4, 8, 16, 256, 512, 1024):
                yield
                mag = jnp.exp(par(0) * float(e))
                pw[e] = (mag * ph[0], mag * ph[1])
            if e in (1, 256, 512, 1024):
                put((1, 256, 512, 1024).index(e), pair, pw[e], pw[e])
            if e == 4:
                w = (par(2), par(3))
                put(4, pair, w, _cmul(w, pw[4]))
            if e == 16:
                put(6, rev, pw[16])
                put(7, first, pw[8], pw[16])
            if e == 256:
                w8 = _cmul((par(2), par(3)), pw[8])
                put(5, pair, w8, _cmul(w8, pw[256]))
            if e < 1024:
                ph = (ph[0] * ph[0] - ph[1] * ph[1], 2.0 * ph[0] * ph[1])
            e *= 2

    def powers(i, slab, emit):
        def ld(k):
            r = pl.multiple_of(32 * (192 * (i // 8) + 64 * slab + 8 * (i % 8)) + 32 * k, 8)
            return base_v[pl.ds(r, 16), :], base_v[pl.ds(r + 16, 16), :]
        z = ld(0)
        p15 = _cmul(ld(4), z)
        yield
        p26 = _cmul(p15, ld(0))
        emit(0, p15, p26)
        yield
        p37 = _cmul(p26, ld(0))
        yield
        p48 = _cmul(p37, ld(0))
        emit(1, p37, p48)
        yield
        z = ld(1)
        emit(2, _cmul(p26, z), _cmul(p48, z))
        yield
        p516 = _cmul(p48, ld(2))
        yield
        emit(3, p516, _cmul(p516, ld(1)))
        yield
        p1032 = _cmul(ld(5), ld(3))
        yield
        emit(4, p1032, _cmul(p1032, ld(2)))
        yield
        qb = None
        for t in range(8):
            qa = ld(7) if t == 0 else _cmul(qb, ld(6))
            yield
            qb = _cmul(qa, ld(6))
            if t == 7:
                keep = lax.broadcasted_iota(jnp.int32, (16, 128), 0) < 12
                qb = (jnp.where(keep, qb[0], 1.0), jnp.where(keep, qb[1], 0.0))
            emit(5 + t, qa, qb)
            yield

    def gen(i, pq_v, pq3_v):
        for hf in range(2):
            def emit(t, a, b, hf=hf):
                for cg in range(2):
                    for c in range(2):
                        pq_v[2 * hf + cg, c, 16 * t:16 * t + 16, :] = _pack(
                            a[c][8 * cg:8 * cg + 8], b[c][8 * cg:8 * cg + 8])
            yield from powers(i, hf, emit)

        def emit2(t, a, b):
            for cg in range(2):
                n = 13 * cg + t
                for c in range(2):
                    tmp_v[n, c] = _pack(a[c][8 * cg:8 * cg + 8], b[c][8 * cg:8 * cg + 8])
                re = tmp_v.bitcast(U32)[n, 0]
                im = pltpu.roll(tmp_v.bitcast(U32)[n, 1], 64, 1)
                pq3_v[cg, 8 * t:8 * t + 8, :] = jnp.where(half, re, im)
                pq3_v[2 + cg, 8 * t:8 * t + 8, :] = jnp.where(half, im, re)
        yield from powers(i, 2, emit2)

    def kgen(hf, pq_v, pq3_v, raw_v, zero, gate):
        def operand(grp, start, size):
            return jnp.concatenate(
                [_rows(pq_v, (grp, 0), start, size), _rows(pq_v, (grp, 1), start, size),
                 pltpu.bitcast(pq3_v[grp, start // 2:(start + size) // 2, :], BF16)], axis=1)
        outs = [lax.dot_general(operand(zero + 2 * hf + cg, 0, 80), operand(zero + 2 * hf + cg, 80, 128), NT_DIMS,
                                preferred_element_type=F32) for cg in range(2)]
        for cg, o in enumerate(outs):
            for g in range(5):
                r = 80 * (2 * hf + cg) + 16 * g
                raw_v[r:r + 16, :] = o[16 * g:16 * g + 16]
                if g in (1, 4):
                    gate(o[16 * g:16 * g + 8])
                    yield

    def extract(i, raw_v):
        for hf in range(2):
            for g in range(5):
                parts = []
                for v in (2 * g, 2 * g + 1):
                    a, b = (raw_v[80 * (2 * hf + cg) + 8 * v:80 * (2 * hf + cg) + 8 * v + 8, :] for cg in range(2))
                    parts += [jnp.where(low, a, b), pltpu.roll(jnp.where(low, b, a), 4, 0)]
                r = [pltpu.roll(p, s_, 1, stride=1, stride_axis=0) for s_, p in enumerate(parts)]
                r = jnp.where(slot < 2, jnp.where(slot == 0, r[0], r[1]), jnp.where(slot == 2, r[2], r[3]))
                kt_v[g, pl.ds(pl.multiple_of(128 * (i // 8) + 64 * hf + 8 * (i % 8), 8), 8), :] = r

    def udft(t, j):
        r = jnp.dot(pltpu.bitcast(f_v[...], BF16), _rows(u_v, (t,), j * 128, 128), preferred_element_type=F32)
        for q in range(0, 256, 64):
            uf_v[pl.ds(pl.multiple_of((t * NB + j) * 256 + q, 8), 64), :] = r[q:q + 64]
            z_v[pl.ds(pl.multiple_of(zero_s[0] + 4 * SLABS, 8), 8), :] = r[q:q + 8]
            yield

    def kdft(t, gate):
        rows = pl.ds(pl.multiple_of(t * 128, 128), 128)
        for m in range(NB):
            acc = None
            for idx, (mm, g) in enumerate(keys):
                if mm == m:
                    r = lax.dot_general(pltpu.bitcast(g_v[idx], BF16), kt_v[g, rows, :].astype(BF16), NT_DIMS,
                                        preferred_element_type=F32)
                    acc = r if acc is None else acc + r
            for q in range(0, 256, 64):
                big_v[pl.ds(pl.multiple_of(KF0 + (t * NB + m) * 256 + q, 8), 64), :] = acc[q:q + 64]
                gate(acc[q:q + 8])
                yield

    def weights(t, k):
        rows = pl.ds(pl.multiple_of(t * 128, 128), 128)
        if k < 3:
            for c in range(NT):
                wt_v[k, 128 * c:128 * (c + 1), :] = w_v[rows, k * D + 128 * c:k * D + 128 * (c + 1)].astype(F32).T
        elif k == 3:
            wt_v[3] = wo_v[:, rows].astype(F32)
        else:
            for d in range(DH):
                v = wt_v[k - 4, pl.ds(d, H, stride=DH), :].astype(BF16)
                if k < 7:
                    wp_v[t, (k - 4) * D + d * H:(k - 4) * D + (d + 1) * H, :] = v
                else:
                    wop_v[t, d * H:(d + 1) * H, :] = v

    f_cp.wait()

    def phase0(t, carry):
        u_cp(t).wait()

        @pl.when(t + 1 < NT)
        def _():
            for c in par_cp(t + 1):
                c.wait()

        @pl.when(t == 1)
        def _():
            for c in late_cp[:3]:
                c.start()
        mxu = _chain(*[udft(t, j) for j in range(NB)])
        side = _chain(*[bases(192 * t + 24 * c, 3) for c in range(8)])
        _run(_interleave(mxu, 4 * NB, side, 8 * 7, lead=2))
        prepare(jnp.minimum(t + 1, NT - 1))
        return carry
    with jax.named_scope("phase0"):
        lax.fori_loop(0, NT, phase0, 0)

    n_grp = D // 16
    bufs = list(zip(pq_refs[0::2], pq_refs[1::2]))
    raws = (rawa_v, rawb_v)
    _run(gen(0, *bufs[0]))
    _run(gen(1, *bufs[1]))
    for c in late_cp[:3]:
        c.wait()

    for c in late_cp[3:]:
        c.start()

    def phase1(t, carry):
        zero = zero_s[0]

        def gate(v):
            base_v[pl.ds(pl.multiple_of(zero + 32 * SLABS, 8), 8), :] = v
        dft = kdft(jnp.maximum(t - 1, 0), gate)
        for k in range(8):
            i = 8 * t + k
            extract(jnp.maximum(i - 1, 0), raws[(k + 1) % 2])
            weights(t, k)
            n_dft = (4, 4, 8, 8, 8, 8, 12, 12)[k]
            mxu = _chain(kgen(0, *bufs[k % 4], raws[k % 2], zero, gate),
                         kgen(1, *bufs[k % 4], raws[k % 2], zero, gate), _take(dft, n_dft))
            side = gen(jnp.minimum(i + 2, n_grp - 1), *bufs[(k + 2) % 4])
            _run(_interleave(mxu, 8 + n_dft, side, 75, lead=0 if k == 0 else 0))
        return carry
    with jax.named_scope("phase1"):
        lax.fori_loop(0, NT, phase1, 0)
    extract(n_grp - 1, raws[(n_grp - 1) % 2])
    _run(kdft(NT - 1, lambda v: None))

    for c in late_cp[3:]:
        c.wait()
    scale = DH ** -0.5 * LOG2E

    def block_products(t, r8, sg):
        def ld(ref, base, m):
            return [ref[pl.ds(pl.multiple_of(base + ((t * NB + m) * 2 + c) * 128 + r8, 8), 8), :] for c in range(2)]
        prev = None
        for c0 in range(0, NB, 2):
            acc, kc = [None, None], {}
            for j in range(c0 + 1, -1, -1):
                u = ld(uf_v, 0, j)
                for c in range(c0 + 1, max(c0, j) - 1, -1):
                    if c - j not in kc:
                        kc[c - j] = ld(big_v, KF0, c - j)
                    p, a = _cmul(kc[c - j], u), acc[c - c0]
                    acc[c - c0] = p if a is None else [x + y for x, y in zip(a, p)]
                    yield
            for c in (c0, c0 + 1):
                cur = yr, yi = acc[c - c0]
                if prev is not None:
                    yr, yi = yr - sg * prev[1], yi + sg * prev[0]
                yf_v[t, c, pl.ds(r8, 8), :] = yr
                yf_v[t, c, pl.ds(r8 + 128, 8), :] = yi
                prev = cur

    def qkv(r0):
        for n0 in range(0, 3 * NT, NBK):
            xb = jnp.concatenate([_rows(x_v, (k,), r0, RB) for k in range(NT)], axis=1)
            w = jnp.concatenate([_rows(wp_v, (k,), 128 * n0, 128 * NBK) for k in range(NT)], axis=1)
            r = lax.dot_general(xb, w, NT_DIMS, preferred_element_type=F32)
            for q in range(0, RB, 16):
                for n in range(n0, n0 + NBK):
                    v = r[q:q + 16, 128 * (n - n0):128 * (n - n0 + 1)]
                    if n < NT:
                        big_v[pl.ds(pl.multiple_of(n * S + r0 + q, 8), 16), :] = v * scale
                    else:
                        (k_v, v_v)[n // NT - 1][n % NT, pl.ds(pl.multiple_of(HALO + r0 + q, 8), 16), :] = v
                        big_v[pl.ds(pl.multiple_of(GATE0 + r0 // 32, 8), 8), :] = v[0:8]
                    yield

    def logits(i):
        lag = 3
        for step in range(RB // 8 + lag):
            n = step
            if n < RB // 8:
                r = pl.multiple_of(i * RB + n * 8, 8)
                a = [None] * WIN
                for t in range(NT):
                    q = big_v[pl.ds(t * S + r, 8), :]
                    for w in range(WIN):
                        qk = q * k_v[t, pl.ds(r + HALO - DIL * w, 8), :]
                        a[w] = qk if t == 0 else a[w] + qk
                    yield
                for w in range(WIN):
                    lg0_v[(n * WIN + w) * 8:(n * WIN + w + 1) * 8, :] = a[w]
            n = step - lag
            if n >= 0:
                for w in range(WIN):
                    a = lg0_v[(n * WIN + w) * 8:(n * WIN + w + 1) * 8, :]
                    lg1_v[pl.ds(pl.multiple_of(i * RB * WIN + (n * WIN + w) * 8, 8), 8), :] = (
                        a + pltpu.roll(a, 64, 1))
            yield

    def phase3(i, carry):
        sg = jnp.where(i < 4, 1.0, -1.0).astype(F32)
        prod = _chain(*[block_products(t, pl.multiple_of(i * 16 + 8 * hf, 8), sg)
                        for t in range(NT) for hf in range(2)])
        lgt, mxu = logits(jnp.maximum(i - 1, 0)), qkv(pl.multiple_of(i * RB, RB))
        n_mxu, n_lgt = NT * RB // 16, 3 * RB // 8 + 2
        for n_prod in (410, 540, 410):
            side = _take(prod, n_prod)
            if n_prod < 540:
                side = _interleave(side, n_prod, _take(lgt, n_lgt), n_lgt)
            _run(_interleave(_take(mxu, n_mxu), n_mxu, side, n_prod))
        _run(_chain(mxu, prod, lgt))
        return carry
    with jax.named_scope("phase3"):
        lax.fori_loop(0, S // RB, phase3, 0)

    def attend(i, o_ref):
        def softmax(n):
            r = pl.multiple_of(i * RB + n * 8, 8)
            sc = []
            for w in range(WIN):
                a = lg1_v[pl.ds(pl.multiple_of(i * RB * WIN + (n * WIN + w) * 8, 8), 8), :]
                a = a + pltpu.roll(a, 32, 1)
                if n * 8 < DIL * w:
                    a = jnp.where(sub + r >= DIL * w, a, -1e9 * LOG2E)
                sc.append(a)
            mx = functools.reduce(jnp.maximum, sc)
            p = [jnp.exp2(a - mx) for a in sc]
            inv = 1.0 / functools.reduce(lambda a, b: a + b, p)
            o = [None] * NT
            for w in range(WIN):
                for t in range(NT):
                    pv = p[w] * v_v[t, pl.ds(r + HALO - DIL * w, 8), :]
                    o[t] = pv if w == 0 else o[t] + pv
            return [v * inv for v in o]

        held = None
        for n in range(RB // 8):
            o = softmax(n)
            if n % 2 == 0:
                held = o
            else:
                for t in range(NT):
                    o_ref[t, 8 * (n - 1):8 * (n + 1), :] = _pack(held[t], o[t])
            yield
    n_att = RB // 8

    def out_copy(i, col, width):
        at = pl.ds(pl.multiple_of(i * RB, RB), RB), pl.ds(col, width)
        return pltpu.make_async_copy(out_v.at[at], out_hbm.at[(0, *at)], osems.at[i])

    def finish(i, o_ref):
        r0 = pl.multiple_of(i * RB, RB)

        def gate(v):
            for ref, base in ((lg1_v, WIN * S),):
                ref[pl.ds(pl.multiple_of(base + 8 * i, 8), 8), :] = v
        for t in range(NT):
            for c2 in range(RB // 128):
                fi = jnp.concatenate([pltpu.bitcast(fi_v[k], BF16) for k in range(2)], axis=1)
                y = jnp.dot(fi, yf_v[t, i * (RB // 128) + c2].astype(BF16), preferred_element_type=F32)
                for q in range(0, 128, 32):
                    rows = pl.ds(pl.multiple_of(r0 + 128 * c2 + q, 32), 32)
                    yq = y[q:q + 32] + u_v[t, rows, :].astype(F32) * gain_v[t, 2:3, :]
                    out_v[rows, D + 128 * t:D + 128 * (t + 1)] = yq.astype(BF16)
                    gate(yq[0:8])
                    yield
        out_copy(i, D, D).start()
        for t in range(NT):
            r = jnp.dot(jnp.concatenate([_rows(o_ref, (k,), 0, RB) for k in range(NT)], axis=1),
                        _rows(wop_v, (t,), 0, D), preferred_element_type=F32)
            for q in range(0, RB, 16):
                out_v[pl.ds(r0 + q, 16), 128 * t:128 * (t + 1)] = r[q:q + 16].astype(BF16)
                gate(r[q:q + 8])
                yield
            out_copy(i, 128 * t, 128).start()
    n_fin = NT * (RB // 16 + 4 * RB // 128)

    _run(logits(S // RB - 1))
    _run(attend(0, oa_v))

    def phase4(it, carry):
        _run(_interleave(finish(2 * it, oa_v), n_fin, attend(2 * it + 1, ob_v), n_att))
        _run(_interleave(finish(2 * it + 1, ob_v), n_fin, attend(jnp.minimum(2 * it + 2, S // RB - 1), oa_v), n_att))
        return carry
    with jax.named_scope("phase4"):
        lax.fori_loop(0, S // RB // 2, phase4, 0)
    for i in range(S // RB):
        out_copy(i, 0, 2 * D).wait()


@jax.jit
def pallas_concat_heads__sliding_local_dilated__ssm_conv_s4__prompt_kernel(
    A_x: jax.Array,
    A_wqkv: jax.Array,
    A_wo: jax.Array,
    B_u: jax.Array,
    B_A_re: jax.Array,
    B_A_im: jax.Array,
    B_B_re: jax.Array,
    B_B_im: jax.Array,
    B_C_re: jax.Array,
    B_C_im: jax.Array,
    B_log_dt: jax.Array,
    B_Dskip: jax.Array,
):
    keys, gt, fwd, inv = _tables()
    hbm = pl.BlockSpec(memory_space=pl.ANY)
    vmem = pl.BlockSpec(memory_space=pltpu.VMEM)
    scratch = [
        pltpu.VMEM((NT, S, 128), BF16),
        pltpu.VMEM((D, 3 * D), BF16),
        pltpu.VMEM((D, D), BF16),
        pltpu.VMEM((NT, S, 128), BF16),
        pltpu.VMEM((NT, 6, N, 128), BF16),
        pltpu.VMEM(gt.shape, U32),
        pltpu.VMEM(fwd.shape, U32),
        pltpu.VMEM(inv.shape, U32),
        pltpu.SemaphoreType.DMA((21,)),
        pltpu.SemaphoreType.DMA((S // RB,)),
        pltpu.SMEM((1,), jnp.int32),
        pltpu.VMEM((NT, 8, 128), F32),
        pltpu.VMEM((320, 128), F32),
        pltpu.VMEM((320, 128), F32),
        pltpu.VMEM((26, 2, 16, 128), BF16),
        pltpu.VMEM((5, D, 128), F32),
        pltpu.VMEM((32 * SLABS + 8, 128), F32),
        pltpu.VMEM((4 * SLABS + 8, 128), F32),
        pltpu.VMEM((NT * NB * 256, 128), F32),
        pltpu.VMEM((BIG_ROWS, 128), F32),
        pltpu.VMEM((NT, NB, 256, 128), F32),
        pltpu.VMEM((4, D, 128), F32),
        pltpu.VMEM((NT, 3 * D, 128), BF16),
        pltpu.VMEM((NT, D, 128), BF16),
        pltpu.VMEM((NT, RB, 128), BF16),
        pltpu.VMEM((NT, RB, 128), BF16),
        pltpu.VMEM((S, 2 * D), BF16),
        pltpu.VMEM((WIN * RB + 64, 128), F32),
        pltpu.VMEM((WIN * S + 64, 128), F32),
        pltpu.VMEM((NT, S + HALO, 128), F32),
        pltpu.VMEM((NT, S + HALO, 128), F32),
    ] + 4 * [
        pltpu.VMEM((4, 2, 208, 128), BF16),
        pltpu.VMEM((4, 104, 128), U32),
    ]
    return pl.pallas_call(
        _kernel,
        in_specs=[hbm] * 10 + [vmem, vmem] + [hbm] * 3,
        out_specs=hbm,
        out_shape=jax.ShapeDtypeStruct((1, S, 2 * D), BF16),
        scratch_shapes=scratch,
        compiler_params=pltpu.CompilerParams(vmem_limit_bytes=110 * 2**20),
    )(A_x, A_wqkv, A_wo, B_u, B_A_re.T, B_A_im.T, B_B_re.T, B_B_im.T, B_C_re.T, B_C_im.T,
      B_log_dt, B_Dskip, gt, fwd, inv)
```

```python
import functools

import jax
import jax.numpy as jnp
import ml_dtypes
import numpy as np
from jax import lax
import jax.experimental.pallas as pl
import jax.experimental.pallas.tpu as pltpu

S = 2048
D = 640
NT = D // 128
N = 192
H, DH = 32, 20
WIN, DIL = 8, 2
NB = S // 128
RB = 256
NBK = 1
LOG2E = float(np.log2(np.e))
HALO = 16

F32 = jnp.float32
BF16 = jnp.bfloat16
U32 = jnp.uint32
NT_DIMS = (((1,), (1,)), ((), ()))

_ALPHA = ((1, 5, 2, 6), (3, 7, 4, 8), (258, 262, 260, 264), (516, 520, 772, 776),
          (1032, 1288, 1544, 1800))


@functools.lru_cache(maxsize=None)
def _tables():
    pos = {}
    for g in range(5):
        for b in range(32):
            for s in range(4):
                pos[_ALPHA[g][s] + 8 * b] = (g, (4 * b + s + 3) % 128)
    kk = np.concatenate([np.arange(0, 128, 2), np.arange(1, 128, 2)])
    th = 2 * np.pi * (kk + 0.5) / 256
    lr = np.arange(S, dtype=np.float32).astype(ml_dtypes.bfloat16).astype(np.int64)
    gm = {}
    for lag in range(1, S):
        m = (lag - 1) // 128
        g, j = pos[int(lr[lag])]
        gm.setdefault((m, g), np.zeros((128, 128), complex))[:, j] += np.exp(-1j * th * (lag - 128 * m))
    keys = tuple(sorted(gm))

    gt = np.stack([np.concatenate([gm[k].real, gm[k].imag]) for k in keys])
    f = np.exp(-1j * th[:, None] * np.arange(128)[None, :])
    fwd = np.concatenate([f.real, f.imag])
    inv = (2.0 / 256) * np.concatenate([f.real, f.imag]).T

    def words(a):
        b = np.asarray(a, np.float32).astype(ml_dtypes.bfloat16).view(np.uint16).astype(np.uint32)
        return b[..., 0::2, :] | (b[..., 1::2, :] << 16)
    return keys, words(gt), words(fwd), words(np.stack([inv[:, :128], inv[:, 128:]]))


def _cmul(a, b):
    return a[0] * b[0] - a[1] * b[1], a[0] * b[1] + a[1] * b[0]


def _interleave(main, n_main, side, n_side, lead=0):
    for _ in range(lead):
        next(side)
    n_side -= lead
    done = 0
    for k, _ in enumerate(main):
        while done * n_main < (k + 1) * n_side:
            next(side, None)
            done += 1
        yield
    _run(side)


def _take(gen, n):
    for _ in range(n):
        next(gen, None)
        yield


def _run(gen):
    for _ in gen:
        pass


def _chain(*gens):
    for g in gens:
        yield from g


def _pack(a, b):
    return jnp.concatenate([a, b], axis=0).astype(BF16)


def _rows(ref, idx, start, size):
    start = start // 2 if isinstance(start, int) else pl.multiple_of(start // 2, 8)
    return pltpu.bitcast(ref.bitcast(U32)[(*idx, pl.ds(start, size // 2), slice(None))], BF16)


SLABS = 3 * D // 2
KF0 = NT * S
GATE0 = KF0 + NT * NB * 256
BIG_ROWS = GATE0 + 8 * (S // RB)


def _kernel(x_hbm, wqkv_hbm, wo_hbm, u_hbm, are_hbm, aim_hbm, bre_hbm, bim_hbm, cre_hbm, cim_hbm,
            ldt_ref, dsk_ref, g_hbm, f_hbm, fi_hbm, out_hbm,
            x_v, w_v, wo_v, u_v, par_v, g_v, f_v, fi_v, sems, osems, zero_s,
            gain_v, rawa_v, rawb_v, tmp_v, kt_v, base_v, z_v, uf_v, big_v, yf_v,
            wt_v, wp_v, wop_v, oa_v, ob_v, out_v, lg0_v, lg1_v, k_v, v_v, *pq_refs):
    keys = _tables()[0]
    zero_s[0] = 0

    def par_cp(t):
        cols = pl.ds(pl.multiple_of(t * 128, 128), 128)
        return [pltpu.make_async_copy(s_.at[:, cols], par_v.at[t, i], sems.at[t]) for i, s_ in enumerate(
            (are_hbm, aim_hbm, bre_hbm, bim_hbm, cre_hbm, cim_hbm))]
    f_cp = pltpu.make_async_copy(f_hbm, f_v, sems.at[6])

    def u_cp(i):
        cols = pl.ds(pl.multiple_of(i * 128, 128), 128)
        return pltpu.make_async_copy(u_hbm.at[0, :, cols], u_v.at[i], sems.at[7 + i])
    late_cp = [pltpu.make_async_copy(a_, b_, sems.at[12 + i]) for i, (a_, b_) in enumerate(
        ((g_hbm, g_v), (wqkv_hbm, w_v), (wo_hbm, wo_v), (fi_hbm, fi_v))
        + tuple((x_hbm.at[0, :, 128 * t:128 * (t + 1)], x_v.at[t]) for t in range(NT)))]
    for c in par_cp(0) + [f_cp, u_cp(0)] + par_cp(1):
        c.start()

    k_v[:, 0:HALO, :] = v_v[:, 0:HALO, :] = jnp.zeros((NT, HALO, 128), F32)
    kt_v[:, 0:128, :] = jnp.zeros((5, 128, 128), F32)
    rawb_v[...] = jnp.zeros(rawb_v.shape, F32)
    dt_row = jnp.exp(ldt_ref[...].astype(F32)).astype(BF16).astype(F32).reshape(1, D)
    skip_row = dsk_ref[...].astype(F32).reshape(1, D)
    for t in range(NT):
        gain_v[t, 0:1, :] = dt_row[:, 128 * t:128 * (t + 1)]
        gain_v[t, 1:2, :] = skip_row[:, 128 * t:128 * (t + 1)]

    def prepare(t):
        dt = gain_v[t, 0:1, :]
        a_re, a_im, b_re, b_im, c_re, c_im = (par_v[t, i].astype(F32) for i in range(6))
        w_re, w_im = _cmul((c_re, c_im), (dt * b_re, dt * b_im))
        gain_v[t, 2:3, :] = jnp.sum(w_re, axis=0, keepdims=True) + gain_v[t, 1:2, :]
        for k, v in enumerate((dt * a_re, dt * a_im, w_re, w_im)):
            r = pl.multiple_of(k * SLABS + 192 * t, 8)
            z_v[pl.ds(r, 128), :] = v[0:128].T
            hi = v[128:].T
            z_v[pl.ds(r + 128, 64), :] = jnp.concatenate([hi[0:64], hi[64:128]], axis=1)

    for c in par_cp(0):
        c.wait()
    for t in range(1, NT):
        for c in [u_cp(t)] + (par_cp(t + 1) if t + 1 < NT else []):
            c.start()
    prepare(0)

    sub = lax.broadcasted_iota(jnp.int32, (8, 128), 0)
    lane = lax.broadcasted_iota(jnp.int32, (8, 128), 1)
    low, half, slot = sub < 4, lane < 64, (lane + 1) % 4

    def sel(a, b):
        return tuple(jnp.where(low, x, y) for x, y in zip(a, b))

    def bases(r0, nv):
        def par(k):
            return z_v[pl.ds(pl.multiple_of(k * SLABS + r0, 8), 8 * nv), :]

        def put(k, fn, *args):
            for n in range(nv):
                v = fn(*[tuple(c[8 * n:8 * n + 8] for c in a) for a in args])
                for cg in range(2):
                    for c in range(2):
                        r = 32 * (r0 + 8 * n) + 8 * (4 * k + 2 * c + cg)
                        base_v[pl.ds(pl.multiple_of(r, 8), 8), :] = v[cg][c]

        def pair(a, b):
            sb = tuple(pltpu.roll(v, 4, 0) for v in b)
            return sel(a, sb), sel(sb, a)

        def rev(a):
            return [tuple(jnp.take_along_axis(v, 4 * cg + 3 - sub % 4, axis=0) for v in (a[0], -a[1]))
                    for cg in range(2)]

        def first(z8, z16):
            z8 = rev(z8)
            return sel((1.0, 0.0), z8[0]), sel(z8[1], rev(z16)[1])

        li = par(1)
        ph = (jnp.cos(li), jnp.sin(li))
        pw = {}
        e = 1
        while e <= 1024:
            if e in (1, 4, 8, 16, 256, 512, 1024):
                yield
                mag = jnp.exp(par(0) * float(e))
                pw[e] = (mag * ph[0], mag * ph[1])
            if e in (1, 256, 512, 1024):
                put((1, 256, 512, 1024).index(e), pair, pw[e], pw[e])
            if e == 4:
                w = (par(2), par(3))
                put(4, pair, w, _cmul(w, pw[4]))
            if e == 16:
                put(6, rev, pw[16])
                put(7, first, pw[8], pw[16])
            if e == 256:
                w8 = _cmul((par(2), par(3)), pw[8])
                put(5, pair, w8, _cmul(w8, pw[256]))
            if e < 1024:
                ph = (ph[0] * ph[0] - ph[1] * ph[1], 2.0 * ph[0] * ph[1])
            e *= 2

    def powers(i, slab, emit):
        def ld(k):
            r = pl.multiple_of(32 * (192 * (i // 8) + 64 * slab + 8 * (i % 8)) + 32 * k, 8)
            return base_v[pl.ds(r, 16), :], base_v[pl.ds(r + 16, 16), :]
        z = ld(0)
        p15 = _cmul(ld(4), z)
        yield
        p26 = _cmul(p15, ld(0))
        emit(0, p15, p26)
        yield
        p37 = _cmul(p26, ld(0))
        yield
        p48 = _cmul(p37, ld(0))
        emit(1, p37, p48)
        yield
        z = ld(1)
        emit(2, _cmul(p26, z), _cmul(p48, z))
        yield
        p516 = _cmul(p48, ld(2))
        yield
        emit(3, p516, _cmul(p516, ld(1)))
        yield
        p1032 = _cmul(ld(5), ld(3))
        yield
        emit(4, p1032, _cmul(p1032, ld(2)))
        yield
        qb = None
        for t in range(8):
            qa = ld(7) if t == 0 else _cmul(qb, ld(6))
            yield
            qb = _cmul(qa, ld(6))
            if t == 7:
                keep = lax.broadcasted_iota(jnp.int32, (16, 128), 0) < 12
                qb = (jnp.where(keep, qb[0], 1.0), jnp.where(keep, qb[1], 0.0))
            emit(5 + t, qa, qb)
            yield

    def gen(i, pq_v, pq3_v):
        for hf in range(2):
            def emit(t, a, b, hf=hf):
                for cg in range(2):
                    for c in range(2):
                        pq_v[2 * hf + cg, c, 16 * t:16 * t + 16, :] = _pack(
                            a[c][8 * cg:8 * cg + 8], b[c][8 * cg:8 * cg + 8])
            yield from powers(i, hf, emit)

        def emit2(t, a, b):
            for cg in range(2):
                n = 13 * cg + t
                for c in range(2):
                    tmp_v[n, c] = _pack(a[c][8 * cg:8 * cg + 8], b[c][8 * cg:8 * cg + 8])
                re = tmp_v.bitcast(U32)[n, 0]
                im = pltpu.roll(tmp_v.bitcast(U32)[n, 1], 64, 1)
                pq3_v[cg, 8 * t:8 * t + 8, :] = jnp.where(half, re, im)
                pq3_v[2 + cg, 8 * t:8 * t + 8, :] = jnp.where(half, im, re)
        yield from powers(i, 2, emit2)

    def kgen(hf, pq_v, pq3_v, raw_v, zero, gate):
        def operand(grp, start, size):
            return jnp.concatenate(
                [_rows(pq_v, (grp, 0), start, size), _rows(pq_v, (grp, 1), start, size),
                 pltpu.bitcast(pq3_v[grp, start // 2:(start + size) // 2, :], BF16)], axis=1)
        outs = [lax.dot_general(operand(zero + 2 * hf + cg, 0, 80), operand(zero + 2 * hf + cg, 80, 128), NT_DIMS,
                                preferred_element_type=F32) for cg in range(2)]
        for cg, o in enumerate(outs):
            for g in range(5):
                r = 80 * (2 * hf + cg) + 16 * g
                raw_v[r:r + 16, :] = o[16 * g:16 * g + 16]
                if g in (1, 4):
                    gate(o[16 * g:16 * g + 8])
                    yield

    def extract(i, raw_v):
        for hf in range(2):
            for g in range(5):
                parts = []
                for v in (2 * g, 2 * g + 1):
                    a, b = (raw_v[80 * (2 * hf + cg) + 8 * v:80 * (2 * hf + cg) + 8 * v + 8, :] for cg in range(2))
                    parts += [jnp.where(low, a, b), pltpu.roll(jnp.where(low, b, a), 4, 0)]
                r = [pltpu.roll(p, s_, 1, stride=1, stride_axis=0) for s_, p in enumerate(parts)]
                r = jnp.where(slot < 2, jnp.where(slot == 0, r[0], r[1]), jnp.where(slot == 2, r[2], r[3]))
                kt_v[g, pl.ds(pl.multiple_of(128 * (i // 8) + 64 * hf + 8 * (i % 8), 8), 8), :] = r

    def udft(t, j):
        r = jnp.dot(pltpu.bitcast(f_v[...], BF16), _rows(u_v, (t,), j * 128, 128), preferred_element_type=F32)
        for q in range(0, 256, 64):
            uf_v[pl.ds(pl.multiple_of((t * NB + j) * 256 + q, 8), 64), :] = r[q:q + 64]
            z_v[pl.ds(pl.multiple_of(zero_s[0] + 4 * SLABS, 8), 8), :] = r[q:q + 8]
            yield

    def kdft(t, gate):
        rows = pl.ds(pl.multiple_of(t * 128, 128), 128)
        for m in range(NB):
            acc = None
            for idx, (mm, g) in enumerate(keys):
                if mm == m:
                    r = lax.dot_general(pltpu.bitcast(g_v[idx], BF16), kt_v[g, rows, :].astype(BF16), NT_DIMS,
                                        preferred_element_type=F32)
                    acc = r if acc is None else acc + r
            for q in range(0, 256, 64):
                big_v[pl.ds(pl.multiple_of(KF0 + (t * NB + m) * 256 + q, 8), 64), :] = acc[q:q + 64]
                gate(acc[q:q + 8])
                yield

    def weights(t, k):
        rows = pl.ds(pl.multiple_of(t * 128, 128), 128)
        if k < 3:
            for c in range(NT):
                wt_v[k, 128 * c:128 * (c + 1), :] = w_v[rows, k * D + 128 * c:k * D + 128 * (c + 1)].astype(F32).T
        elif k == 3:
            wt_v[3] = wo_v[:, rows].astype(F32)
        else:
            for d in range(DH):
                v = wt_v[k - 4, pl.ds(d, H, stride=DH), :].astype(BF16)
                if k < 7:
                    wp_v[t, (k - 4) * D + d * H:(k - 4) * D + (d + 1) * H, :] = v
                else:
                    wop_v[t, d * H:(d + 1) * H, :] = v

    f_cp.wait()

    def phase0(t, carry):
        u_cp(t).wait()

        @pl.when(t + 1 < NT)
        def _():
            for c in par_cp(t + 1):
                c.wait()

        @pl.when(t == 1)
        def _():
            for c in late_cp[:3]:
                c.start()
        mxu = _chain(*[udft(t, j) for j in range(NB)])
        side = _chain(*[bases(192 * t + 24 * c, 3) for c in range(8)])
        _run(_interleave(mxu, 4 * NB, side, 8 * 7, lead=2))
        prepare(jnp.minimum(t + 1, NT - 1))
        return carry
    with jax.named_scope("phase0"):
        lax.fori_loop(0, NT, phase0, 0)

    n_grp = D // 16
    bufs = list(zip(pq_refs[0::2], pq_refs[1::2]))
    raws = (rawa_v, rawb_v)
    _run(gen(0, *bufs[0]))
    _run(gen(1, *bufs[1]))
    for c in late_cp[:3]:
        c.wait()

    for c in late_cp[3:]:
        c.start()

    def phase1(t, carry):
        zero = zero_s[0]

        def gate(v):
            base_v[pl.ds(pl.multiple_of(zero + 32 * SLABS, 8), 8), :] = v
        dft = kdft(jnp.maximum(t - 1, 0), gate)
        for k in range(8):
            i = 8 * t + k
            extract(jnp.maximum(i - 1, 0), raws[(k + 1) % 2])
            weights(t, k)
            n_dft = (4, 4, 8, 8, 8, 8, 12, 12)[k]
            mxu = _chain(kgen(0, *bufs[k % 4], raws[k % 2], zero, gate),
                         kgen(1, *bufs[k % 4], raws[k % 2], zero, gate), _take(dft, n_dft))
            side = gen(jnp.minimum(i + 2, n_grp - 1), *bufs[(k + 2) % 4])
            _run(_interleave(mxu, 8 + n_dft, side, 75, lead=0 if k == 0 else 0))
        return carry
    with jax.named_scope("phase1"):
        lax.fori_loop(0, NT, phase1, 0)
    extract(n_grp - 1, raws[(n_grp - 1) % 2])
    _run(kdft(NT - 1, lambda v: None))

    for c in late_cp[3:]:
        c.wait()
    scale = DH ** -0.5 * LOG2E

    def block_products(t, r8, sg):
        def ld(ref, base, m):
            return [ref[pl.ds(pl.multiple_of(base + ((t * NB + m) * 2 + c) * 128 + r8, 8), 8), :] for c in range(2)]
        prev = None
        for c0 in range(0, NB, 2):
            acc, kc = [None, None], {}
            for j in range(c0 + 1, -1, -1):
                u = ld(uf_v, 0, j)
                for c in range(c0 + 1, max(c0, j) - 1, -1):
                    if c - j not in kc:
                        kc[c - j] = ld(big_v, KF0, c - j)
                    p, a = _cmul(kc[c - j], u), acc[c - c0]
                    acc[c - c0] = p if a is None else [x + y for x, y in zip(a, p)]
                    yield
            for c in (c0, c0 + 1):
                cur = yr, yi = acc[c - c0]
                if prev is not None:
                    yr, yi = yr - sg * prev[1], yi + sg * prev[0]
                yf_v[t, c, pl.ds(r8, 8), :] = yr
                yf_v[t, c, pl.ds(r8 + 128, 8), :] = yi
                prev = cur

    def qkv(r0):
        for n0 in range(0, 3 * NT, NBK):
            xb = jnp.concatenate([_rows(x_v, (k,), r0, RB) for k in range(NT)], axis=1)
            w = jnp.concatenate([_rows(wp_v, (k,), 128 * n0, 128 * NBK) for k in range(NT)], axis=1)
            r = lax.dot_general(xb, w, NT_DIMS, preferred_element_type=F32)
            for q in range(0, RB, 16):
                for n in range(n0, n0 + NBK):
                    v = r[q:q + 16, 128 * (n - n0):128 * (n - n0 + 1)]
                    if n < NT:
                        big_v[pl.ds(pl.multiple_of(n * S + r0 + q, 8), 16), :] = v * scale
                    else:
                        (k_v, v_v)[n // NT - 1][n % NT, pl.ds(pl.multiple_of(HALO + r0 + q, 8), 16), :] = v
                        big_v[pl.ds(pl.multiple_of(GATE0 + r0 // 32, 8), 8), :] = v[0:8]
                    yield

    def logits(i):
        lag = 3
        for step in range(RB // 8 + lag):
            n = step
            if n < RB // 8:
                r = pl.multiple_of(i * RB + n * 8, 8)
                a = [None] * WIN
                for t in range(NT):
                    q = big_v[pl.ds(t * S + r, 8), :]
                    for w in range(WIN):
                        qk = q * k_v[t, pl.ds(r + HALO - DIL * w, 8), :]
                        a[w] = qk if t == 0 else a[w] + qk
                    yield
                for w in range(WIN):
                    lg0_v[(n * WIN + w) * 8:(n * WIN + w + 1) * 8, :] = a[w]
            n = step - lag
            if n >= 0:
                for w in range(WIN):
                    a = lg0_v[(n * WIN + w) * 8:(n * WIN + w + 1) * 8, :]
                    lg1_v[pl.ds(pl.multiple_of(i * RB * WIN + (n * WIN + w) * 8, 8), 8), :] = (
                        a + pltpu.roll(a, 64, 1))
            yield

    def phase3(i, carry):
        sg = jnp.where(i < 4, 1.0, -1.0).astype(F32)
        prod = _chain(*[block_products(t, pl.multiple_of(i * 16 + 8 * hf, 8), sg)
                        for t in range(NT) for hf in range(2)])
        _run(_interleave(qkv(pl.multiple_of(i * RB, RB)), 3 * NT * RB // 16, prod, 10 * 136))
        return carry
    with jax.named_scope("phase3"):
        lax.fori_loop(0, S // RB, phase3, 0, unroll=2)

    def attend(i, o_ref):
        def softmax(n):
            r = pl.multiple_of(i * RB + n * 8, 8)
            sc = []
            for w in range(WIN):
                a = lg1_v[pl.ds(pl.multiple_of(i * RB * WIN + (n * WIN + w) * 8, 8), 8), :]
                a = a + pltpu.roll(a, 32, 1)
                if n * 8 < DIL * w:
                    a = jnp.where(sub + r >= DIL * w, a, -1e9 * LOG2E)
                sc.append(a)
            mx = functools.reduce(jnp.maximum, sc)
            p = [jnp.exp2(a - mx) for a in sc]
            inv = 1.0 / functools.reduce(lambda a, b: a + b, p)
            o = [None] * NT
            for w in range(WIN):
                for t in range(NT):
                    pv = p[w] * v_v[t, pl.ds(r + HALO - DIL * w, 8), :]
                    o[t] = pv if w == 0 else o[t] + pv
            return [v * inv for v in o]

        held = None
        for n in range(RB // 8):
            o = softmax(n)
            if n % 2 == 0:
                held = o
            else:
                for t in range(NT):
                    o_ref[t, 8 * (n - 1):8 * (n + 1), :] = _pack(held[t], o[t])
            yield
    n_att = RB // 8

    def out_copy(i, col, width):
        at = pl.ds(pl.multiple_of(i * RB, RB), RB), pl.ds(col, width)
        return pltpu.make_async_copy(out_v.at[at], out_hbm.at[(0, *at)], osems.at[i])

    def idft(i):
        r0 = pl.multiple_of(i * RB, RB)
        for t in range(NT):
            for c2 in range(RB // 128):
                fi = jnp.concatenate([pltpu.bitcast(fi_v[k], BF16) for k in range(2)], axis=1)
                y = jnp.dot(fi, yf_v[t, i * (RB // 128) + c2].astype(BF16), preferred_element_type=F32)
                for q in range(0, 128, 32):
                    rows = pl.ds(pl.multiple_of(r0 + 128 * c2 + q, 32), 32)
                    yq = y[q:q + 32] + u_v[t, rows, :].astype(F32) * gain_v[t, 2:3, :]
                    out_v[rows, D + 128 * t:D + 128 * (t + 1)] = yq.astype(BF16)
                    yield
        out_copy(i, D, D).start()

    def project(i, o_ref):
        r0 = pl.multiple_of(i * RB, RB)
        for t in range(NT):
            r = jnp.dot(jnp.concatenate([_rows(o_ref, (k,), 0, RB) for k in range(NT)], axis=1),
                        _rows(wop_v, (t,), 0, D), preferred_element_type=F32)
            for q in range(0, RB, 16):
                out_v[pl.ds(r0 + q, 16), 128 * t:128 * (t + 1)] = r[q:q + 16].astype(BF16)
                lg1_v[pl.ds(pl.multiple_of(WIN * S + 8 * i, 8), 8), :] = r[q:q + 8]
                yield
            out_copy(i, 128 * t, 128).start()
    n_fin = NT * RB // 16

    def phase3b(i, carry):
        _run(_interleave(idft(i), 40, logits(i), 6 * RB // 8 + 3))
        return carry
    with jax.named_scope("phase3b"):
        lax.fori_loop(0, S // RB, phase3b, 0)
    _run(attend(0, oa_v))

    def phase4(it, carry):
        _run(_interleave(project(2 * it, oa_v), n_fin, attend(2 * it + 1, ob_v), n_att, lead=3))
        _run(_interleave(project(2 * it + 1, ob_v), n_fin, attend(jnp.minimum(2 * it + 2, S // RB - 1), oa_v), n_att))
        return carry
    with jax.named_scope("phase4"):
        lax.fori_loop(0, S // RB // 2, phase4, 0)
    for i in range(S // RB):
        out_copy(i, 0, 2 * D).wait()


@jax.jit
def pallas_concat_heads__sliding_local_dilated__ssm_conv_s4__prompt_kernel(
    A_x: jax.Array,
    A_wqkv: jax.Array,
    A_wo: jax.Array,
    B_u: jax.Array,
    B_A_re: jax.Array,
    B_A_im: jax.Array,
    B_B_re: jax.Array,
    B_B_im: jax.Array,
    B_C_re: jax.Array,
    B_C_im: jax.Array,
    B_log_dt: jax.Array,
    B_Dskip: jax.Array,
):
    keys, gt, fwd, inv = _tables()
    hbm = pl.BlockSpec(memory_space=pl.ANY)
    vmem = pl.BlockSpec(memory_space=pltpu.VMEM)
    scratch = [
        pltpu.VMEM((NT, S, 128), BF16),
        pltpu.VMEM((D, 3 * D), BF16),
        pltpu.VMEM((D, D), BF16),
        pltpu.VMEM((NT, S, 128), BF16),
        pltpu.VMEM((NT, 6, N, 128), BF16),
        pltpu.VMEM(gt.shape, U32),
        pltpu.VMEM(fwd.shape, U32),
        pltpu.VMEM(inv.shape, U32),
        pltpu.SemaphoreType.DMA((21,)),
        pltpu.SemaphoreType.DMA((S // RB,)),
        pltpu.SMEM((1,), jnp.int32),
        pltpu.VMEM((NT, 8, 128), F32),
        pltpu.VMEM((320, 128), F32),
        pltpu.VMEM((320, 128), F32),
        pltpu.VMEM((26, 2, 16, 128), BF16),
        pltpu.VMEM((5, D, 128), F32),
        pltpu.VMEM((32 * SLABS + 8, 128), F32),
        pltpu.VMEM((4 * SLABS + 8, 128), F32),
        pltpu.VMEM((NT * NB * 256, 128), F32),
        pltpu.VMEM((BIG_ROWS, 128), F32),
        pltpu.VMEM((NT, NB, 256, 128), F32),
        pltpu.VMEM((4, D, 128), F32),
        pltpu.VMEM((NT, 3 * D, 128), BF16),
        pltpu.VMEM((NT, D, 128), BF16),
        pltpu.VMEM((NT, RB, 128), BF16),
        pltpu.VMEM((NT, RB, 128), BF16),
        pltpu.VMEM((S, 2 * D), BF16),
        pltpu.VMEM((WIN * RB + 64, 128), F32),
        pltpu.VMEM((WIN * S + 64, 128), F32),
        pltpu.VMEM((NT, S + HALO, 128), F32),
        pltpu.VMEM((NT, S + HALO, 128), F32),
    ] + 4 * [
        pltpu.VMEM((4, 2, 208, 128), BF16),
        pltpu.VMEM((4, 104, 128), U32),
    ]
    return pl.pallas_call(
        _kernel,
        in_specs=[hbm] * 10 + [vmem, vmem] + [hbm] * 3,
        out_specs=hbm,
        out_shape=jax.ShapeDtypeStruct((1, S, 2 * D), BF16),
        scratch_shapes=scratch,
        compiler_params=pltpu.CompilerParams(vmem_limit_bytes=110 * 2**20),
    )(A_x, A_wqkv, A_wo, B_u, B_A_re.T, B_A_im.T, B_B_re.T, B_B_im.T, B_C_re.T, B_C_im.T,
      B_log_dt, B_Dskip, gt, fwd, inv)
```
